```python
import jax
import jax.numpy as jnp

def _softmax(x, axis=-1):
    return jax.nn.softmax(x, axis=axis)
def _gelu(x):
    return jax.nn.gelu(x, approximate=True)
def _silu(x):
    return jax.nn.silu(x)
def _sigmoid(x):
    return jax.nn.sigmoid(x)
def _layernorm(x, axis=-1, eps=1e-5):
    m = jnp.mean(x, axis=axis, keepdims=True)
    v = jnp.var(x, axis=axis, keepdims=True)
    return (x - m) / jnp.sqrt(v + eps)
def _scatter_add(tgt, idx, src, axis=0):
    return tgt.at[idx].add(src)
def _segment_sum(src, seg, n):
    return jax.ops.segment_sum(src, seg, n)
class _Rng:
    def __init__(self, key):
        self._k = key
    def _next(self):
        self._k, sub = jax.random.split(self._k)
        return sub
    def normal(self, shape):
        return jax.random.normal(self._next(), shape, dtype=jnp.bfloat16)
    def randint(self, lo, hi, shape):
        return jax.random.randint(self._next(), shape, lo, hi, dtype=jnp.int32)
    def uniform(self, shape, lo=0.0, hi=1.0):
        return jax.random.uniform(self._next(), shape, jnp.bfloat16, lo, hi)
    def permutation(self, n):
        return jax.random.permutation(self._next(), n)


kernel_name = 'concat_heads__compressed_kv_cla__spectral_gfnet__prompt'

def setup_inputs():
    _rng = _Rng(jax.random.key(int.from_bytes(__import__("os").urandom(4), "little")))
    _w = (lambda a: (lambda t: t.astype(jnp.bfloat16) if jnp.issubdtype(t.dtype, jnp.floating) else t)(jnp.asarray(a)))
    def _A_setup():
        B, H, Sq, Sk, D, M = 1, 32, 2048, 2048, 128, 1024
        Dc = 4 * D
        return {
            "x": _w((lambda *s: _rng.normal(s) * 0.05)(B, Sq, M)),
            "c_kv": _w((lambda *s: _rng.normal(s) * 0.05)(B, Sk, Dc)),
            "w_q": _w((lambda *s: _rng.normal(s) * 0.05)(M, H, D) * (M ** -0.5)),
            "w_uk": _w((lambda *s: _rng.normal(s) * 0.05)(Dc, H, D) * (Dc ** -0.5)),
            "w_uv": _w((lambda *s: _rng.normal(s) * 0.05)(Dc, H, D) * (Dc ** -0.5)),
            "w_o": _w((lambda *s: _rng.normal(s) * 0.05)(H, D, M) * ((H * D) ** -0.5)),
        }
    _A_in = _A_setup()

    def _B_setup():
        B, S, D = 1, 2048, 1024
        Df = D // 2 + 1
        return {
            "x": _w((lambda *s: _rng.normal(s) * 0.05)(B, S, D)),
            "w_r": _w((lambda *s: _rng.normal(s) * 0.05)(S, Df) * 0.02),
            "w_i": _w((lambda *s: _rng.normal(s) * 0.05)(S, Df) * 0.02),
        }
    _B_in = _B_setup()

    return {
        "A_x": _A_in["x"],
        "A_c_kv": _A_in["c_kv"],
        "A_w_q": _A_in["w_q"],
        "A_w_uk": _A_in["w_uk"],
        "A_w_uv": _A_in["w_uv"],
        "A_w_o": _A_in["w_o"],
        "B_x": _B_in["x"],
        "B_w_r": _B_in["w_r"],
        "B_w_i": _B_in["w_i"],
    }

def reference(A_x, A_c_kv, A_w_q, A_w_uk, A_w_uv, A_w_o, B_x, B_w_r, B_w_i):
    def _A_ref(x, c_kv, w_q, w_uk, w_uv, w_o):
        B, Sq, M = x.shape[0], x.shape[1], x.shape[2]
        Sk = c_kv.shape[1]
        H, D = w_q.shape[1], w_q.shape[2]
        q = jnp.einsum("bqm,mhd->bhqd", x, w_q)
        k = jnp.einsum("bkc,chd->bhkd", c_kv, w_uk)
        v = jnp.einsum("bkc,chd->bhkd", c_kv, w_uv)
        scores = jnp.einsum("bhqd,bhkd->bhqk", q, k) * (D ** -0.5)
        off = Sk - Sq
        qi = jnp.arange(Sq)[:, None]
        kj = jnp.arange(Sk)[None, :]
        cmask = kj <= (qi + off)
        scores = jnp.where(cmask[None, None], scores, -1e9)
        p = _softmax(scores, axis=-1)
        ctx = jnp.einsum("bhqk,bhkd->bhqd", p, v)
        return jnp.einsum("bhqd,hdm->bqm", ctx, w_o)

    def _B_ref(x, w_r, w_i):
        B, S, D = x.shape
        X = (lambda x, axes=(-2,-1): jnp.fft.rfft2(x.astype(jnp.float32), axes=axes))(x, axes=(-2, -1))
        W = w_r + 1j * w_i
        X = X * W
        y = (lambda x, s, axes=(-2,-1): jnp.fft.irfft2(x, s=s, axes=axes).astype(jnp.bfloat16))(X, (S, D), axes=(-2, -1))
        return y

    a = _A_ref(A_x, A_c_kv, A_w_q, A_w_uk, A_w_uv, A_w_o)
    b = _B_ref(B_x, B_w_r, B_w_i)
    return jnp.concatenate([a, b], axis=-1)
```

```python
import functools
import numpy as np
import jax
import jax.numpy as jnp
from jax import lax
from jax.experimental import pallas as pl
from jax.experimental.pallas import tpu as pltpu

S = 2048; D = 128; H = 32; M = 1024; C = 512; DM = 1024
NT = (((1,), (1,)), ((), ()))
NEG = -1e30
LOG2E = 1.4426950408889634
F32 = jnp.float32; BF16 = jnp.bfloat16


def bf(x): return pltpu.bitcast(x, BF16)

def _kset(j):
    cA, cB = (0, 4) if j == 0 else (j, 8 - j)
    e = np.arange(64)
    return np.concatenate([cA + 8 * e, cB + 8 * e])


def _bf16_np(a):
    import ml_dtypes
    return np.asarray(a, dtype=np.float32).astype(ml_dtypes.bfloat16)


def _consts():
    b = np.arange(128); alt = (-1.0) ** b
    FT = np.zeros((4, 272, 256)); G = np.zeros((4, 256, 256))
    for j in range(4):
        k = _kset(j)
        th = 2 * np.pi * np.outer(k, b) / 1024
        cw = (np.where(k == 0, 1.0, 2.0) / 1024)[:, None]
        if j == 0:
            A = (k % 8 == 0)[:, None]
            FT[0, :128, :128] = np.where(A, np.cos(th), 0); FT[0, :128, 128:] = np.where(~A, np.cos(th), 0)
            FT[0, 128:256, :128] = np.where(A, -np.sin(th), 0); FT[0, 128:256, 128:] = np.where(~A, -np.sin(th), 0)
            FT[0, 256, :128] = alt
            G[0, :128, :128] = np.where(A, cw * np.cos(th), 0); G[0, 128:, :128] = np.where(A, -cw * np.sin(th), 0)
            G[0, :128, 128:] = np.where(~A, cw * np.cos(th), 0); G[0, 128:, 128:] = np.where(~A, -cw * np.sin(th), 0)
            G[0, 128, :128] = alt / 1024
        else:
            s = np.where(k % 8 == j, 1.0, -1.0)[:, None]
            FT[j, :128, :128] = np.cos(th); FT[j, :128, 128:] = s * np.sin(th)
            FT[j, 128:256, :128] = -np.sin(th); FT[j, 128:256, 128:] = s * np.cos(th)
            G[j, :128, :128] = cw * np.cos(th); G[j, 128:, :128] = -cw * np.sin(th)
            G[j, :128, 128:] = s * cw * np.sin(th); G[j, 128:, 128:] = s * cw * np.cos(th)
    Ma = np.zeros((16, 256, 256)); Mi = np.zeros((16, 256, 256))
    for a in range(16):
        E = np.exp(-2j * np.pi * np.outer(a + 16 * b, b) / 2048)
        Ma[a] = np.block([[E.real, E.imag], [-E.imag, E.real]])
        Ci = np.conj(E) / 2048
        Mi[a] = np.block([[Ci.real, -Ci.imag], [Ci.imag, Ci.real]])
    FTb = FT.reshape(4, 272, 2, 128).transpose(0, 2, 1, 3)
    Gb = G.reshape(4, 256, 2, 128).transpose(0, 2, 1, 3)
    Mab = Ma.reshape(16, 256, 2, 128).transpose(0, 2, 1, 3)
    Mib = Mi.reshape(16, 256, 2, 128).transpose(0, 2, 1, 3)
    return _bf16_np(FTb), _bf16_np(Gb), _bf16_np(Mab), _bf16_np(Mib)


def _r4(x0, x1, x2, x3, inverse):
    t0 = (x0[0] + x2[0], x0[1] + x2[1]); t1 = (x0[0] - x2[0], x0[1] - x2[1])
    t2 = (x1[0] + x3[0], x1[1] + x3[1]); t3 = (x1[0] - x3[0], x1[1] - x3[1])
    y0 = (t0[0] + t2[0], t0[1] + t2[1]); y2 = (t0[0] - t2[0], t0[1] - t2[1])
    a = (t1[0] + t3[1], t1[1] - t3[0])
    b = (t1[0] - t3[1], t1[1] + t3[0])
    return (y0, b, y2, a) if inverse else (y0, a, y2, b)


def _tw(x, m, inverse):
    m = m % 16
    if m == 0: return x
    xr, xi = x
    sg = -1.0 if inverse else 1.0
    if m == 4:
        return (xi, -xr) if not inverse else (-xi, xr)
    r = float(np.sqrt(0.5))
    if m == 2:
        if not inverse: return ((xr + xi) * r, (xi - xr) * r)
        return ((xr - xi) * r, (xi + xr) * r)
    if m == 6:
        if not inverse: return ((xi - xr) * r, (xr + xi) * (-r))
        return ((xr + xi) * (-r), (xr - xi) * r)
    c = float(np.cos(2 * np.pi * m / 16)); s = float(np.sin(2 * np.pi * m / 16)) * sg
    return (xr * c + xi * s, xi * c - xr * s)


def fft16(xs, inverse):
    A = [None] * 4
    for n2 in range(4):
        ys = _r4(xs[n2], xs[4 + n2], xs[8 + n2], xs[12 + n2], inverse)
        A[n2] = [_tw(ys[k1], n2 * k1, inverse) for k1 in range(4)]
    out = [None] * 16
    for k1 in range(4):
        ys = _r4(A[0][k1], A[1][k1], A[2][k1], A[3][k1], inverse)
        for k2 in range(4):
            out[k1 + 4 * k2] = ys[k2]
    return out


def attention_steps(qi, ki, vi, ctx, slot, h, bq, bk):
    def ld(ref, r0, r1): return bf(ref[slot, r0 // 2:r1 // 2, :])
    nq = S // bq

    def tiles(i):
        out = []; k0 = 0
        while k0 < i * bq:
            k1 = min(k0 + bk, i * bq); out.append((k0, k1, 0)); k0 = k1
        for t in range(bq // 128):
            out.append((i * bq + t * 128, i * bq + (t + 1) * 128, t * 128))
        return out
    state = {'ms': None, 'sl': []}
    sts = {}
    steps = []

    def qk(i, tile):
        def f():
            k0, k1, r0 = tile
            s = lax.dot_general(ld(qi, i * bq + r0, (i + 1) * bq), ld(ki, k0, k1), NT, preferred_element_type=F32)
            if k1 > i * bq:
                row = lax.broadcasted_iota(jnp.int32, (128, 128), 0)
                col = lax.broadcasted_iota(jnp.int32, (128, 128), 1)
                top = jnp.where(col <= row, s[:128], NEG)
                s = jnp.concatenate([top, s[128:]], axis=0) if s.shape[0] > 128 else top
            state['sl'].append(s)
            mx = s[:, :128]
            for c in range(1, (k1 - k0) // 128):
                mx = jnp.maximum(mx, s[:, c * 128:(c + 1) * 128])
            ms = state['ms']
            if ms is None: state['ms'] = mx
            elif r0 == 0: state['ms'] = jnp.maximum(ms, mx)
            else: state['ms'] = jnp.concatenate([ms[:r0], jnp.maximum(ms[r0:], mx)], axis=0)
        return f

    def begin(i):
        def f():
            sts[i] = {'m': jnp.max(state['ms'], axis=1, keepdims=True), 'l': None, 'acc': None, 's': state['sl']}
            state['sl'] = []; state['ms'] = None
        return f

    def pv(i, tile, j):
        def f():
            st = sts[i]; s = st['s'][j]
            k0, k1, r0 = tile
            p = jnp.exp2(s - st['m'][r0:])
            ls = p[:, :128]
            for c in range(1, (k1 - k0) // 128):
                ls = ls + p[:, c * 128:(c + 1) * 128]
            o = jnp.dot(p.astype(BF16), ld(vi, k0, k1), preferred_element_type=F32)
            if st['l'] is None: st['l'] = ls; st['acc'] = o
            elif r0 == 0: st['l'] = st['l'] + ls; st['acc'] = st['acc'] + o
            else:
                st['l'] = jnp.concatenate([st['l'][:r0], st['l'][r0:] + ls], axis=0)
                st['acc'] = jnp.concatenate([st['acc'][:r0], st['acc'][r0:] + o], axis=0)
        return f

    def fin(i):
        def f():
            st = sts[i]
            l = jnp.sum(st['l'], axis=1, keepdims=True)
            r = pltpu.reciprocal(l, approx=True); r = r * (2.0 - l * r)
            ctx[h, i * bq:(i + 1) * bq, :] = (st['acc'] * r).astype(BF16)
        return f
    for t in tiles(0): steps.append((('qk', 0), qk(0, t)))
    for i in range(nq):
        steps.append((('begin', i), begin(i)))
        tn = tiles(i + 1) if i + 1 < nq else []; tc = tiles(i)
        for j in range(max(len(tn), len(tc))):
            if j < len(tn): steps.append((('qk', i + 1), qk(i + 1, tn[j])))
            if j < len(tc): steps.append((('pv', i, j), pv(i, tc[j], j)))
        steps.append((('fin', i), fin(i)))
    return steps


def proj_steps(hn, slot, xi, ci, wc, wslot, qb, kb, vb, rc):
    sh = ((1 - (hn & 1)) * 16).astype(jnp.uint32)

    def half(w32): return pltpu.bitcast((w32 << sh) & jnp.uint32(0xffff0000), F32).astype(BF16)
    st = {}
    steps = []

    def getw():
        if 'wq' not in st:
            st['wq'] = half(wc[wslot, 0:M, :])
            st['wkv'] = jnp.concatenate([half(wc[wslot, M:M + C, :]), half(wc[wslot, M + C:, :])], axis=1)

    def qchunk(r):
        def f():
            getw()
            lhs = jnp.concatenate([bf(xi[j, r * rc // 2:(r + 1) * rc // 2, :]) for j in range(M // 128)], axis=1)
            q = jnp.dot(lhs, st['wq'], preferred_element_type=F32) * (D ** -0.5 * LOG2E)
            qb[slot, r * rc:(r + 1) * rc, :] = q.astype(BF16)
        return f

    def kvchunk(r):
        def f():
            getw()
            lhs = jnp.concatenate([bf(ci[j, r * rc // 2:(r + 1) * rc // 2, :]) for j in range(C // 128)], axis=1)
            kv = jnp.dot(lhs, st['wkv'], preferred_element_type=F32)
            kb[slot, r * rc:(r + 1) * rc, :] = kv[:, :D].astype(BF16)
            vb[slot, r * rc:(r + 1) * rc, :] = kv[:, D:].astype(BF16)
        return f
    for r in range(S // rc):
        steps.append(kvchunk(r)); steps.append(qchunk(r))
    return steps


def kernel(x_hbm, c_hbm, wq_hbm, wk_hbm, wv_hbm, wo_hbm, bx_hbm, wr_hbm, wi_hbm, f_hbm, g_hbm, ma_hbm, mi_hbm,
           out_hbm,
           xs, cs, wc, qb, kb, vb, ctx, wos, bxs, wr32, wi32, wn, x1r, x1i, vr, vi_, tr, ti, y1r, y1i,
           fs, gs, mas, mis, ost,
           sem, wsem, osem, *, UR, bq, bk, rc, RO, NPV, NTAIL, FINAT, FIN7):
    def cp(src, dst, s): return pltpu.make_async_copy(src, dst, s)
    bx_u = bx_hbm.bitcast(jnp.uint32)
    bx_cp = [cp(bx_u.at[:, m, :], bxs.at[m], sem.at[m]) for m in range(8)]
    f_cp = cp(f_hbm, fs, sem.at[8])
    ma_cp = cp(ma_hbm, mas, sem.at[9])
    mi_cp = cp(mi_hbm, mis, sem.at[10])
    g_cp = cp(g_hbm, gs, sem.at[11])
    wr_u = wr_hbm.at[pl.ds(0, 512), :].bitcast(jnp.uint32)
    wi_u = wi_hbm.at[pl.ds(0, 512), :].bitcast(jnp.uint32)
    w_cp = [cp(wr_u.at[:, cc * 128:(cc + 1) * 128], wr32.at[cc], sem.at[36 + cc]) for cc in range(16)]
    w_cp += [cp(wi_u.at[:, cc * 128:(cc + 1) * 128], wi32.at[cc], sem.at[52 + cc]) for cc in range(16)]
    wn_cp = [cp(wr_hbm.at[pl.ds(512, 1), :], wn.at[0], sem.at[12]), cp(wi_hbm.at[pl.ds(512, 1), :], wn.at[1], sem.at[13])]
    x_cp = [cp(x_hbm.at[:, a * 128:(a + 1) * 128], xs.at[a], sem.at[14 + a]) for a in range(8)]
    c_cp = [cp(c_hbm.at[:, a * 128:(a + 1) * 128], cs.at[a], sem.at[22 + a]) for a in range(4)]
    wo_cp = [cp(wo_hbm.at[:, a * 128:(a + 1) * 128], wos.at[a], sem.at[26 + a]) for a in range(8)]
    wq_u = wq_hbm.bitcast(jnp.uint32); wk_u = wk_hbm.bitcast(jnp.uint32); wv_u = wv_hbm.bitcast(jnp.uint32)

    def w_cps(j, wslot):
        return [cp(wq_u.at[:, j, :], wc.at[wslot, pl.ds(0, M), :], wsem.at[wslot, 0]),
                cp(wk_u.at[:, j, :], wc.at[wslot, pl.ds(M, C), :], wsem.at[wslot, 1]),
                cp(wv_u.at[:, j, :], wc.at[wslot, pl.ds(M + C, C), :], wsem.at[wslot, 2])]
    f_cp.start()
    for d in bx_cp: d.start()
    ma_cp.start()
    for d in w_cp + wn_cp: d.start()
    mi_cp.start(); g_cp.start()
    for d in c_cp + x_cp: d.start()
    for d in w_cps(0, 0): d.start()
    for d in wo_cp: d.start()

    fi = fs.bitcast(jnp.int32); gi = gs.bitcast(jnp.int32)
    mai = mas.bitcast(jnp.int32); mii = mis.bitcast(jnp.int32)
    x1ri = x1r.bitcast(jnp.int32); x1ii = x1i.bitcast(jnp.int32)
    tri = tr.bitcast(jnp.int32); tii = ti.bitcast(jnp.int32)
    r2 = float(np.sqrt(0.5))
    HI = jnp.uint32(0xffff0000)
    for a in range(16):
        tr[a, pl.ds(528, 112), :] = jnp.zeros((112, 128), BF16)
        ti[a, pl.ds(528, 112), :] = jnp.zeros((112, 128), BF16)
        x1i[a, pl.ds(512, 16), :] = jnp.zeros((16, 128), BF16)
    f_cp.wait()
    for m in range(8):
        bx_cp[m].wait()
        for par in range(2):
            a = 2 * m + par
            xa = []
            for A in range(8):
                w = bxs[m, :, A * 128:(A + 1) * 128]
                xa.append(pltpu.bitcast(w << 16 if par == 0 else w & HI, F32))
            u0, u1 = xa[0] + xa[4], xa[0] - xa[4]; u2, u3 = xa[2] + xa[6], xa[2] - xa[6]
            u4, u5 = xa[1] + xa[5], xa[1] - xa[5]; u6, u7 = xa[3] + xa[7], xa[3] - xa[7]
            s_, t_ = u0 + u2, u4 + u6
            d57, s57 = (u5 - u7) * r2, (u5 + u7) * r2
            L = [(s_ + t_, s_ - t_), (u1 + d57, (u3 + s57) * -1.0), (u0 - u2, u6 - u4), (u1 - d57, u3 - s57)]
            for j in range(4):
                data = jnp.concatenate(L[j], axis=1).astype(BF16)
                nr = 272 if j == 0 else 256
                lhs = jnp.concatenate([bf(fi[j, 0, 0:nr // 2, :]), bf(fi[j, 1, 0:nr // 2, :])], axis=1)
                o = lax.dot_general(lhs, data, NT, preferred_element_type=F32).astype(BF16)
                x1r[a, j * 128:(j + 1) * 128, :] = o[:128]
                x1i[a, j * 128:(j + 1) * 128, :] = o[128:256]
                if j == 0:
                    x1r[a, 512:528, :] = o[256:272]

    ma_cp.wait()
    for a in range(16):
        lhs = jnp.concatenate([bf(x1ri[a]), bf(x1ii[a])], axis=1)
        rhs = jnp.concatenate([bf(mai[a, 0]), bf(mai[a, 1])], axis=1)
        o = jnp.dot(lhs, rhs, preferred_element_type=F32)
        vr[a] = o[:, :128]
        vi_[a] = o[:, 128:]

    for d in w_cp + wn_cp: d.wait()

    def mid_unit(k0, wload):
        xs_ = [(vr[a, k0:k0 + UR, :], vi_[a, k0:k0 + UR, :]) for a in range(16)]
        X = fft16(xs_, False)
        Y = []
        for cc in range(16):
            wr_, wi_ = wload(cc)
            xr, xi_2 = X[cc]
            Y.append((xr * wr_ - xi_2 * wi_, xr * wi_ + xi_2 * wr_))
        Tt = fft16(Y, True)
        for a in range(16):
            tr[a, k0:k0 + UR, :] = Tt[a][0].astype(BF16)
            ti[a, k0:k0 + UR, :] = Tt[a][1].astype(BF16)
    for j in range(4):
        for hf in range(2):
            c = (0, 4)[hf] if j == 0 else (j, 8 - j)[hf]
            for g in range(64 // UR):
                e0 = g * UR

                def wload(cc, c=c, e0=e0):
                    wr_ = wr32[cc, pl.ds(c // 2 + 4 * e0, UR, stride=4), :]
                    wi_ = wi32[cc, pl.ds(c // 2 + 4 * e0, UR, stride=4), :]
                    if c % 2 == 0:
                        return pltpu.bitcast(wr_ << 16, F32), pltpu.bitcast(wi_ << 16, F32)
                    return pltpu.bitcast(wr_ & HI, F32), pltpu.bitcast(wi_ & HI, F32)
                mid_unit(j * 128 + hf * 64 + e0, wload)

    def wload_n(cc):
        return (jnp.broadcast_to(wn[0, :, cc * 128:(cc + 1) * 128].astype(F32), (UR, 128)),
                jnp.broadcast_to(wn[1, :, cc * 128:(cc + 1) * 128].astype(F32), (UR, 128)))
    mid_unit(512, wload_n)

    mi_cp.wait()
    for a in range(16):
        lhs = jnp.concatenate([bf(mii[a, 0]), bf(mii[a, 1])], axis=1)
        data = jnp.concatenate([bf(tri[a]), bf(tii[a])], axis=1)
        o = lax.dot_general(lhs, data, NT, preferred_element_type=F32)
        y1r[a] = o[:128]
        y1i[a] = o[128:, :512]

    g_cp.wait()
    out_u = out_hbm.bitcast(jnp.uint32)
    b_out = [cp(bxs.at[m], out_u.at[:, m, pl.ds(DM, DM)], osem.at[m]) for m in range(8)]
    lane = lax.broadcasted_iota(jnp.int32, (128, 128), 1)
    for m in range(8):
        ys = []
        for par in range(2):
            a = 2 * m + par
            U = []
            for j in range(4):
                yr = y1r[a, :, j * 128:(j + 1) * 128]; yi = y1i[a, :, j * 128:(j + 1) * 128]
                if j == 0:
                    yi = jnp.where(lane == 0, y1r[a, :, 512:640], yi)
                lhs = jnp.concatenate([yr, yi], axis=1).astype(BF16)
                rhs = jnp.concatenate([bf(gi[j, 0]), bf(gi[j, 1])], axis=1)
                o = jnp.dot(lhs, rhs, preferred_element_type=F32)
                U.append((o[:, :128], o[:, 128:]))
            T0, T4 = U[0]; U1r, U1i = U[1]; U2r, U2i = U[2]; U3r, U3i = U[3]
            P, Q = T0 + T4, T0 - T4
            A_, B_ = P + U2r, P - U2r
            s13 = U1r + U3r; d = U3i - U1i
            Qm, Qp = Q - U2i, Q + U2i
            t1, t2 = U1r - U3r, U1i + U3i
            e1, e3 = (t1 - t2) * r2, (t1 + t2) * r2
            ys.append([A_ + s13, Qm + e1, B_ + d, Qp - e3, A_ - s13, Qm - e1, B_ - d, Qp + e3])
        for A in range(8):
            bxs[m, :, A * 128:(A + 1) * 128] = pltpu.bitcast(
                pltpu.pack_elementwise([ys[0][A], ys[1][A]], packed_dtype=BF16), jnp.uint32)
        b_out[m].start()

    xi = xs.bitcast(jnp.int32); ci = cs.bitcast(jnp.int32)
    qi = qb.bitcast(jnp.int32); ki = kb.bitcast(jnp.int32); vi = vb.bitcast(jnp.int32)
    for d in c_cp + x_cp: d.wait()
    for d in w_cps(0, 0): d.wait()
    for d in w_cps(1, 1): d.start()
    for f in proj_steps(jnp.int32(0), 0, xi, ci, wc, 0, qb, kb, vb, rc): f()

    def body(h, _):
        slot = h & 1
        hn = jnp.minimum(h + 1, H - 1)
        jn = hn >> 1
        wslot = jn & 1

        @pl.when((h & 1) == 1)
        def _():
            @pl.when(h < H - 1)
            def _():
                for d in w_cps(jn, wslot): d.wait()

            @pl.when(h < H - 3)
            def _():
                for d in w_cps(jn + 1, 1 - wslot): d.start()
        att = attention_steps(qi, ki, vi, ctx, slot, h, bq, bk)
        proj = proj_steps(hn, 1 - slot, xi, ci, wc, wslot, qb, kb, vb, rc)
        fins = {tag[1]: f for tag, f in att if tag[0] == 'fin'}
        nq = S // bq
        pi = 0
        for tag, f in att:
            if tag[0] == 'fin': continue
            f()
            if tag[0] == 'pv' and tag[1] == nq - 1:
                for _ in range(NPV):
                    if pi < len(proj) - NTAIL:
                        proj[pi]()
                        if pi == FINAT:
                            for i_ in range(nq - 1): fins[i_]()
                        pi += 1
        k_ = 0
        while pi < len(proj):
            proj[pi](); pi += 1; k_ += 1
            if k_ == FIN7: fins[nq - 1]()
        if k_ < FIN7: fins[nq - 1]()
        return 0
    lax.fori_loop(0, H, body, 0)

    for d in wo_cp: d.wait()
    for d_ in b_out: d_.wait()
    ctxi = ctx.bitcast(jnp.int32); woi = wos.bitcast(jnp.int32)

    def a_out_cps(r16, osl):
        return [cp(ost.at[osl, a], out_hbm.at[pl.ds(r16, RO // 16), :, pl.ds(a * 128, 128)], osem.at[8 + osl * 8 + a]) for a in range(8)]

    def obody(r, _):
        r0 = r * (RO // 16); h0 = pl.multiple_of(r * (RO // 2), RO // 2)
        osl = r & 1

        @pl.when(r >= 2)
        def _():
            for d_ in a_out_cps(r0 - 2 * (RO // 16), osl): d_.wait()
        lhs = jnp.concatenate([bf(ctxi[hh, pl.ds(h0, RO // 2), :]) for hh in range(H)], axis=1)
        rhs = jnp.concatenate([bf(woi[a]) for a in range(8)], axis=1)
        o = jnp.dot(lhs, rhs, preferred_element_type=F32)
        for a in range(8):
            ost[osl, a] = o[:, a * 128:(a + 1) * 128].astype(BF16).reshape(RO // 16, 16, 128)
        for d_ in a_out_cps(r0, osl): d_.start()
        return 0
    lax.fori_loop(0, S // RO, obody, 0)
    for r in (S // RO - 2, S // RO - 1):
        for d_ in a_out_cps(r * (RO // 16), r & 1): d_.wait()


def make_fn(UR=16, bq=256, bk=256, rc=256, RO=256, NPV=2, NTAIL=2, FINAT=3, FIN7=1):
    FTb, Gb, Mab, Mib = _consts()

    def fn(A_x, A_c_kv, A_w_q, A_w_uk, A_w_uv, A_w_o, B_x, B_w_r, B_w_i):
        x = A_x.reshape(S, M); c = A_c_kv.reshape(S, C); wo = A_w_o.reshape(H * D, M)
        bx = B_x.reshape(128, 16, DM)
        out = pl.pallas_call(
            functools.partial(kernel, UR=UR, bq=bq, bk=bk, rc=rc, RO=RO, NPV=NPV, NTAIL=NTAIL, FINAT=FINAT, FIN7=FIN7),
            in_specs=[pl.BlockSpec(memory_space=pl.ANY)] * 13,
            out_specs=pl.BlockSpec(memory_space=pl.ANY),
            out_shape=jax.ShapeDtypeStruct((128, 16, M + DM), BF16),
            scratch_shapes=[
                pltpu.VMEM((M // 128, S, 128), BF16),
                pltpu.VMEM((C // 128, S, 128), BF16),
                pltpu.VMEM((2, M + 2 * C, D), jnp.uint32),
                pltpu.VMEM((2, S, D), BF16), pltpu.VMEM((2, S, D), BF16), pltpu.VMEM((2, S, D), BF16),
                pltpu.VMEM((H, S, D), BF16),
                pltpu.VMEM((8, H * D, 128), BF16),
                pltpu.VMEM((8, 128, DM), jnp.uint32),
                pltpu.VMEM((16, 256, 128), jnp.uint32), pltpu.VMEM((16, 256, 128), jnp.uint32),
                pltpu.VMEM((2, 1, S), BF16),
                pltpu.VMEM((16, 528, 128), BF16), pltpu.VMEM((16, 528, 128), BF16),
                pltpu.VMEM((16, 528, 128), F32), pltpu.VMEM((16, 528, 128), F32),
                pltpu.VMEM((16, 640, 128), BF16), pltpu.VMEM((16, 640, 128), BF16),
                pltpu.VMEM((16, 128, 640), F32), pltpu.VMEM((16, 128, 512), F32),
                pltpu.VMEM((4, 2, 272, 128), BF16), pltpu.VMEM((4, 2, 256, 128), BF16),
                pltpu.VMEM((16, 2, 256, 128), BF16), pltpu.VMEM((16, 2, 256, 128), BF16),
                pltpu.VMEM((2, 8, RO // 16, 16, 128), BF16),
                pltpu.SemaphoreType.DMA((68,)), pltpu.SemaphoreType.DMA((2, 3)), pltpu.SemaphoreType.DMA((24,)),
            ],
            compiler_params=pltpu.CompilerParams(vmem_limit_bytes=126 * 2 ** 20),
        )(x, c, A_w_q, A_w_uk, A_w_uv, wo, bx, B_w_r.T, B_w_i.T,
          jnp.asarray(FTb), jnp.asarray(Gb), jnp.asarray(Mab), jnp.asarray(Mib))
        return out.reshape(1, S, M + DM)
    return fn


_fn = make_fn()


@jax.jit
def pallas_concat_heads__compressed_kv_cla__spectral_gfnet__prompt_kernel(
    A_x: jax.Array,
    A_c_kv: jax.Array,
    A_w_q: jax.Array,
    A_w_uk: jax.Array,
    A_w_uv: jax.Array,
    A_w_o: jax.Array,
    B_x: jax.Array,
    B_w_r: jax.Array,
    B_w_i: jax.Array,
):
    return _fn(A_x, A_c_kv, A_w_q, A_w_uk, A_w_uv, A_w_o, B_x, B_w_r, B_w_i)
```

```python
import functools
import numpy as np
import jax
import jax.numpy as jnp
from jax import lax
from jax.experimental import pallas as pl
from jax.experimental.pallas import tpu as pltpu

S = 2048; D = 128; H = 32; M = 1024; C = 512; DM = 1024
NT = (((1,), (1,)), ((), ()))
NEG = -1e30
LOG2E = 1.4426950408889634
F32 = jnp.float32; BF16 = jnp.bfloat16


def bf(x): return pltpu.bitcast(x, BF16)

def _kset(j):
    cA, cB = (0, 4) if j == 0 else (j, 8 - j)
    e = np.arange(64)
    return np.concatenate([cA + 8 * e, cB + 8 * e])


def _bf16_np(a):
    import ml_dtypes
    return np.asarray(a, dtype=np.float32).astype(ml_dtypes.bfloat16)


def _consts():
    b = np.arange(128); alt = (-1.0) ** b
    FT = np.zeros((4, 272, 256)); G = np.zeros((4, 256, 256))
    for j in range(4):
        k = _kset(j)
        th = 2 * np.pi * np.outer(k, b) / 1024
        cw = (np.where(k == 0, 1.0, 2.0) / 1024)[:, None]
        if j == 0:
            A = (k % 8 == 0)[:, None]
            FT[0, :128, :128] = np.where(A, np.cos(th), 0); FT[0, :128, 128:] = np.where(~A, np.cos(th), 0)
            FT[0, 128:256, :128] = np.where(A, -np.sin(th), 0); FT[0, 128:256, 128:] = np.where(~A, -np.sin(th), 0)
            FT[0, 256, :128] = alt
            G[0, :128, :128] = np.where(A, cw * np.cos(th), 0); G[0, 128:, :128] = np.where(A, -cw * np.sin(th), 0)
            G[0, :128, 128:] = np.where(~A, cw * np.cos(th), 0); G[0, 128:, 128:] = np.where(~A, -cw * np.sin(th), 0)
            G[0, 128, :128] = alt / 1024
        else:
            s = np.where(k % 8 == j, 1.0, -1.0)[:, None]
            FT[j, :128, :128] = np.cos(th); FT[j, :128, 128:] = s * np.sin(th)
            FT[j, 128:256, :128] = -np.sin(th); FT[j, 128:256, 128:] = s * np.cos(th)
            G[j, :128, :128] = cw * np.cos(th); G[j, 128:, :128] = -cw * np.sin(th)
            G[j, :128, 128:] = s * cw * np.sin(th); G[j, 128:, 128:] = s * cw * np.cos(th)
    G = G / 2048
    E = np.exp(-2j * np.pi * np.outer(b, b) / 128)
    F128 = np.stack([E.real, E.imag]).astype(np.float32)
    TW = np.exp(-2j * np.pi * np.outer(np.arange(16), b) / 2048)
    TW = np.concatenate([TW.real, TW.imag]).astype(np.float32)
    FTb = FT.reshape(4, 272, 2, 128).transpose(0, 2, 1, 3)
    Gb = G.reshape(4, 256, 2, 128).transpose(0, 2, 1, 3)
    return _bf16_np(FTb), _bf16_np(Gb), F128, TW


def _r4(x0, x1, x2, x3, inverse):
    t0 = (x0[0] + x2[0], x0[1] + x2[1]); t1 = (x0[0] - x2[0], x0[1] - x2[1])
    t2 = (x1[0] + x3[0], x1[1] + x3[1]); t3 = (x1[0] - x3[0], x1[1] - x3[1])
    y0 = (t0[0] + t2[0], t0[1] + t2[1]); y2 = (t0[0] - t2[0], t0[1] - t2[1])
    a = (t1[0] + t3[1], t1[1] - t3[0])
    b = (t1[0] - t3[1], t1[1] + t3[0])
    return (y0, b, y2, a) if inverse else (y0, a, y2, b)


def _tw(x, m, inverse):
    m = m % 16
    if m == 0: return x
    xr, xi = x
    sg = -1.0 if inverse else 1.0
    if m == 4:
        return (xi, -xr) if not inverse else (-xi, xr)
    r = float(np.sqrt(0.5))
    if m == 2:
        if not inverse: return ((xr + xi) * r, (xi - xr) * r)
        return ((xr - xi) * r, (xi + xr) * r)
    if m == 6:
        if not inverse: return ((xi - xr) * r, (xr + xi) * (-r))
        return ((xr + xi) * (-r), (xr - xi) * r)
    c = float(np.cos(2 * np.pi * m / 16)); s = float(np.sin(2 * np.pi * m / 16)) * sg
    return (xr * c + xi * s, xi * c - xr * s)


def fft16(xs, inverse):
    A = [None] * 4
    for n2 in range(4):
        ys = _r4(xs[n2], xs[4 + n2], xs[8 + n2], xs[12 + n2], inverse)
        A[n2] = [_tw(ys[k1], n2 * k1, inverse) for k1 in range(4)]
    out = [None] * 16
    for k1 in range(4):
        ys = _r4(A[0][k1], A[1][k1], A[2][k1], A[3][k1], inverse)
        for k2 in range(4):
            out[k1 + 4 * k2] = ys[k2]
    return out


def attention_steps(qi, ki, vi, ctx, slot, h, bq, bk):
    def ld(ref, r0, r1): return bf(ref[slot, r0 // 2:r1 // 2, :])
    nq = S // bq

    def tiles(i):
        out = []; k0 = 0
        while k0 < i * bq:
            k1 = min(k0 + bk, i * bq); out.append((k0, k1, 0)); k0 = k1
        for t in range(bq // 128):
            out.append((i * bq + t * 128, i * bq + (t + 1) * 128, t * 128))
        return out
    state = {'ms': None, 'sl': []}
    sts = {}
    steps = []

    def qk(i, tile):
        def f():
            k0, k1, r0 = tile
            s = lax.dot_general(ld(qi, i * bq + r0, (i + 1) * bq), ld(ki, k0, k1), NT, preferred_element_type=F32)
            if k1 > i * bq:
                row = lax.broadcasted_iota(jnp.int32, (128, 128), 0)
                col = lax.broadcasted_iota(jnp.int32, (128, 128), 1)
                top = jnp.where(col <= row, s[:128], NEG)
                s = jnp.concatenate([top, s[128:]], axis=0) if s.shape[0] > 128 else top
            state['sl'].append(s)
            mx = s[:, :128]
            for c in range(1, (k1 - k0) // 128):
                mx = jnp.maximum(mx, s[:, c * 128:(c + 1) * 128])
            ms = state['ms']
            if ms is None: state['ms'] = mx
            elif r0 == 0: state['ms'] = jnp.maximum(ms, mx)
            else: state['ms'] = jnp.concatenate([ms[:r0], jnp.maximum(ms[r0:], mx)], axis=0)
        return f

    def begin(i):
        def f():
            sts[i] = {'m': jnp.max(state['ms'], axis=1, keepdims=True), 'l': None, 'acc': None, 's': state['sl']}
            state['sl'] = []; state['ms'] = None
        return f

    def pv(i, tile, j):
        def f():
            st = sts[i]; s = st['s'][j]
            k0, k1, r0 = tile
            p = jnp.exp2(s - st['m'][r0:])
            ls = jnp.sum(p, axis=1, keepdims=True)
            o = jnp.dot(p.astype(BF16), ld(vi, k0, k1), preferred_element_type=F32)
            if st['l'] is None: st['l'] = ls; st['acc'] = o
            elif r0 == 0: st['l'] = st['l'] + ls; st['acc'] = st['acc'] + o
            else:
                st['l'] = jnp.concatenate([st['l'][:r0], st['l'][r0:] + ls], axis=0)
                st['acc'] = jnp.concatenate([st['acc'][:r0], st['acc'][r0:] + o], axis=0)
        return f

    def fin(i):
        def f():
            st = sts[i]
            l = st['l']
            r = pltpu.reciprocal(l, approx=True); r = r * (2.0 - l * r)
            ctx[h, i * bq:(i + 1) * bq, :] = (st['acc'] * r).astype(BF16)
        return f
    for t in tiles(0): steps.append((('qk', 0), qk(0, t)))
    for i in range(nq):
        steps.append((('begin', i), begin(i)))
        tn = tiles(i + 1) if i + 1 < nq else []; tc = tiles(i)
        for j in range(max(len(tn), len(tc))):
            if j < len(tn): steps.append((('qk', i + 1), qk(i + 1, tn[j])))
            if j < len(tc): steps.append((('pv', i, j), pv(i, tc[j], j)))
        steps.append((('fin', i), fin(i)))
    return steps


def proj_steps(par, slot, xi, ci, wc, wslot, qb, kb, vb, rc):
    def half(w32):
        w = (w32 << 16) if par == 0 else (w32 & jnp.uint32(0xffff0000))
        return pltpu.bitcast(w, F32).astype(BF16)
    st = {}
    steps = []

    def getw():
        if 'wq' not in st:
            st['wq'] = half(wc[wslot, 0:M, :])
            st['wkv'] = jnp.concatenate([half(wc[wslot, M:M + C, :]), half(wc[wslot, M + C:, :])], axis=1)

    def qchunk(r):
        def f():
            getw()
            lhs = jnp.concatenate([bf(xi[j, r * rc // 2:(r + 1) * rc // 2, :]) for j in range(M // 128)], axis=1)
            q = jnp.dot(lhs, st['wq'], preferred_element_type=F32) * (D ** -0.5 * LOG2E)
            qb[slot, r * rc:(r + 1) * rc, :] = q.astype(BF16)
        return f

    def kvchunk(r):
        def f():
            getw()
            lhs = jnp.concatenate([bf(ci[j, r * rc // 2:(r + 1) * rc // 2, :]) for j in range(C // 128)], axis=1)
            kv = jnp.dot(lhs, st['wkv'], preferred_element_type=F32)
            kb[slot, r * rc:(r + 1) * rc, :] = kv[:, :D].astype(BF16)
            vb[slot, r * rc:(r + 1) * rc, :] = kv[:, D:].astype(BF16)
        return f
    for r in range(S // rc):
        steps.append(kvchunk(r)); steps.append(qchunk(r))
    return steps


SCOPES = False
_stack = []
def begin_scope(n):
    if SCOPES:
        sc = jax.named_scope(n); sc.__enter__(); _stack.append(sc)
def end_scope():
    if SCOPES:
        _stack.pop().__exit__(None, None, None)


def b_steps(R, UR):
    r2 = float(np.sqrt(0.5))
    HI = jnp.uint32(0xffff0000)
    fi = R.fs.bitcast(jnp.int32); gi = R.gs.bitcast(jnp.int32); mai = R.mas.bitcast(jnp.int32)
    x1ri = R.x1r.bitcast(jnp.int32); x1ii = R.x1i.bitcast(jnp.int32)

    def p1(a):
        m, par = a // 2, a % 2

        def f():
            xa = []
            for A in range(8):
                w = R.bxs[m, :, A * 128:(A + 1) * 128]
                xa.append(pltpu.bitcast(w << 16 if par == 0 else w & HI, F32))
            u0, u1 = xa[0] + xa[4], xa[0] - xa[4]; u2, u3 = xa[2] + xa[6], xa[2] - xa[6]
            u4, u5 = xa[1] + xa[5], xa[1] - xa[5]; u6, u7 = xa[3] + xa[7], xa[3] - xa[7]
            s_, t_ = u0 + u2, u4 + u6
            d57, s57 = (u5 - u7) * r2, (u5 + u7) * r2
            L = [(s_ + t_, s_ - t_), (u1 + d57, (u3 + s57) * -1.0), (u0 - u2, u6 - u4), (u1 - d57, u3 - s57)]
            for j in range(4):
                data = jnp.concatenate(L[j], axis=1).astype(BF16)
                nr = 272 if j == 0 else 256
                lhs = jnp.concatenate([bf(fi[j, 0, 0:nr // 2, :]), bf(fi[j, 1, 0:nr // 2, :])], axis=1)
                o = lax.dot_general(lhs, data, NT, preferred_element_type=F32).astype(BF16)
                R.x1r[a, j * 128:(j + 1) * 128, :] = o[:128]
                R.x1i[a, j * 128:(j + 1) * 128, :] = o[128:256]
                if j == 0:
                    R.x1r[a, 512:528, :] = o[256:272]
        return f

    def p2(a, k0, k1):
        def f():
            lhs = jnp.concatenate([bf(x1ri[a, k0 // 2:k1 // 2, :]), bf(x1ii[a, k0 // 2:k1 // 2, :])], axis=1)
            rhs = jnp.concatenate([bf(mai[a, 0]), bf(mai[a, 1])], axis=1)
            o = jnp.dot(lhs, rhs, preferred_element_type=F32)
            for t in range(k0 // 128, (k1 + 127) // 128):
                l0 = max(k0, t * 128); l1 = min(k1, (t + 1) * 128)
                R.vt[t][0, a, l0 - t * 128:l1 - t * 128, :] = o[l0 - k0:l1 - k0, :128]
                R.vt[t][1, a, l0 - t * 128:l1 - t * 128, :] = o[l0 - k0:l1 - k0, 128:]
        return f

    def mid(k0):
        if k0 < 512:
            j, rem = k0 // 128, k0 % 128
            hf, e0 = rem // 64, rem % 64
            c = (0, 4)[hf] if j == 0 else (j, 8 - j)[hf]

            def wload(cc):
                wr_ = R.wr32[cc, pl.ds(c // 2 + 4 * e0, UR, stride=4), :]
                wi_ = R.wi32[cc, pl.ds(c // 2 + 4 * e0, UR, stride=4), :]
                if c % 2 == 0:
                    return pltpu.bitcast(wr_ << 16, F32), pltpu.bitcast(wi_ << 16, F32)
                return pltpu.bitcast(wr_ & HI, F32), pltpu.bitcast(wi_ & HI, F32)
        else:
            def wload(cc):
                return (jnp.broadcast_to(R.wn[0, :, cc * 128:(cc + 1) * 128].astype(F32), (UR, 128)),
                        jnp.broadcast_to(R.wn[1, :, cc * 128:(cc + 1) * 128].astype(F32), (UR, 128)))

        def f():
            t, kk = k0 // 128, k0 % 128
            xs_ = [(R.vt[t][R.z0, a, kk:kk + UR, :], R.vt[t][R.z0 + 1, a, kk:kk + UR, :]) for a in range(16)]
            X = fft16(xs_, False)
            Y = []
            for cc in range(16):
                wr_, wi_ = wload(cc)
                xr, xi_2 = X[cc]
                Y.append((xr * wr_ - xi_2 * wi_, xr * wi_ + xi_2 * wr_))
            Tt = fft16(Y, True)
            for a in range(16):
                R.vt[t][2, a, kk:kk + UR, :] = Tt[a][0]
                R.vt[t][3, a, kk:kk + UR, :] = Tt[a][1]
        return f

    def p3(a, t):
        def f():
            lhs = jnp.concatenate([bf(mai[a, 0]), bf(mai[a, 1])], axis=1)
            data = jnp.concatenate([R.vt[t][2, a], R.vt[t][3, a]], axis=1).astype(BF16)
            o = lax.dot_general(lhs, data, NT, preferred_element_type=F32)
            R.y1r[a, :, t * 128:(t + 1) * 128] = o[:128]
            if t < 4:
                R.y1i[a, :, t * 128:(t + 1) * 128] = o[128:]
        return f

    lane = lax.broadcasted_iota(jnp.int32, (128, 128), 1)
    st = {}

    def p4(a):
        def f():
            U = []
            for j in range(4):
                yr = R.y1r[a, :, j * 128:(j + 1) * 128]; yi = R.y1i[a, :, j * 128:(j + 1) * 128]
                if j == 0:
                    yi = jnp.where(lane == 0, R.y1r[a, :, 512:640], yi)
                lhs = jnp.concatenate([yr, yi], axis=1).astype(BF16)
                rhs = jnp.concatenate([bf(gi[j, 0]), bf(gi[j, 1])], axis=1)
                o = jnp.dot(lhs, rhs, preferred_element_type=F32)
                U.append((o[:, :128], o[:, 128:]))
            T0, T4 = U[0]; U1r, U1i = U[1]; U2r, U2i = U[2]; U3r, U3i = U[3]
            P, Q = T0 + T4, T0 - T4
            A_, B_ = P + U2r, P - U2r
            s13 = U1r + U3r; d = U3i - U1i
            Qm, Qp = Q - U2i, Q + U2i
            t1, t2 = U1r - U3r, U1i + U3i
            e1, e3 = (t1 - t2) * r2, (t1 + t2) * r2
            st[a] = [A_ + s13, Qm + e1, B_ + d, Qp - e3, A_ - s13, Qm - e1, B_ - d, Qp + e3]
            if a % 2 == 1:
                m = a // 2
                for A in range(8):
                    R.bxs[m, :, A * 128:(A + 1) * 128] = pltpu.bitcast(
                        pltpu.pack_elementwise([st[a - 1][A], st[a][A]], packed_dtype=BF16), jnp.uint32)
                R.b_out[m].start()
        return f
    return p1, p2, mid, p3, p4


class NS:
    pass


def kernel(z_ref, x_hbm, c_hbm, wq_hbm, wk_hbm, wv_hbm, wo_hbm, bx_hbm, wr_hbm, wi_hbm, f_hbm, g_hbm, e_hbm, tw_hbm,
           out_hbm,
           xs, cs, wc, qb, kb, vb, ctx, wos, bxs, wr32, wi32, wn, x1r, x1i, vt, y1r, y1i,
           fs, gs, mas, es, tws, ost,
           sem, wsem, osem, *, UR, bq, bk, rc, RO, border, doA=True):
    def cp(src, dst, s): return pltpu.make_async_copy(src, dst, s)
    bx_u = bx_hbm.bitcast(jnp.uint32)
    bx_cp = [cp(bx_u.at[:, m, :], bxs.at[m], sem.at[m]) for m in range(8)]
    f_cp = cp(f_hbm, fs, sem.at[8])
    e_cp = [cp(e_hbm, es, sem.at[9]), cp(tw_hbm, tws, sem.at[10])]
    g_cp = cp(g_hbm, gs, sem.at[11])
    wr_u = wr_hbm.at[pl.ds(0, 512), :].bitcast(jnp.uint32)
    wi_u = wi_hbm.at[pl.ds(0, 512), :].bitcast(jnp.uint32)
    w_cp = [cp(wr_u.at[:, cc * 128:(cc + 1) * 128], wr32.at[cc], sem.at[36 + cc]) for cc in range(16)]
    w_cp += [cp(wi_u.at[:, cc * 128:(cc + 1) * 128], wi32.at[cc], sem.at[52 + cc]) for cc in range(16)]
    wn_cp = [cp(wr_hbm.at[pl.ds(512, 1), :], wn.at[0], sem.at[12]), cp(wi_hbm.at[pl.ds(512, 1), :], wn.at[1], sem.at[13])]
    x_cp = [cp(x_hbm.at[:, a * 128:(a + 1) * 128], xs.at[a], sem.at[14 + a]) for a in range(8)]
    c_cp = [cp(c_hbm.at[:, a * 128:(a + 1) * 128], cs.at[a], sem.at[22 + a]) for a in range(4)]
    wo_cp = [cp(wo_hbm.at[:, a * 128:(a + 1) * 128], wos.at[a], sem.at[26 + a]) for a in range(8)]
    wq_u = wq_hbm.bitcast(jnp.uint32); wk_u = wk_hbm.bitcast(jnp.uint32); wv_u = wv_hbm.bitcast(jnp.uint32)
    out_u = out_hbm.bitcast(jnp.uint32)
    b_out = [cp(bxs.at[m], out_u.at[:, m, pl.ds(DM, DM)], osem.at[m]) for m in range(8)]

    def w_cps(j, wslot):
        return [cp(wq_u.at[:, j, :], wc.at[wslot, pl.ds(0, M), :], wsem.at[wslot, 0]),
                cp(wk_u.at[:, j, :], wc.at[wslot, pl.ds(M, C), :], wsem.at[wslot, 1]),
                cp(wv_u.at[:, j, :], wc.at[wslot, pl.ds(M + C, C), :], wsem.at[wslot, 2])]
    R = NS()
    R.z0 = z_ref[0]
    R.fs, R.gs, R.mas, R.x1r, R.x1i, R.vt = fs, gs, mas, x1r, x1i, vt
    R.bxs, R.wr32, R.wi32, R.wn, R.y1r, R.y1i, R.b_out = bxs, wr32, wi32, wn, y1r, y1i, b_out
    p1, p2, mid, p3, p4 = b_steps(R, UR)

    xi = xs.bitcast(jnp.int32); ci = cs.bitcast(jnp.int32)
    qi = qb.bitcast(jnp.int32); ki = kb.bitcast(jnp.int32); vi = vb.bitcast(jnp.int32)
    proj0 = proj_steps(0, 0, xi, ci, wc, 0, qb, kb, vb, rc)

    def start(ds): return lambda: [d.start() for d in ds]
    def wait(ds): return lambda: [d.wait() for d in ds]

    def zero_init():
        for a in range(16):
            vt[4][2, a, pl.ds(16, 112), :] = jnp.zeros((112, 128), F32)
            vt[4][3, a, pl.ds(16, 112), :] = jnp.zeros((112, 128), F32)
            x1i[a, pl.ds(512, 16), :] = jnp.zeros((16, 128), BF16)
    def gen_ma():
        for d in e_cp: d.wait()
        fr = es[0]; fi_ = es[1]
        for a in range(16):
            tr_ = jnp.broadcast_to(tws[a:a + 1, :], (128, 128)); ti_ = jnp.broadcast_to(tws[16 + a:17 + a, :], (128, 128))
            er = fr * tr_ - fi_ * ti_
            ei = fr * ti_ + fi_ * tr_
            erb = er.astype(BF16)
            mas[a, 0, 0:128, :] = erb
            mas[a, 1, 128:256, :] = erb
            mas[a, 1, 0:128, :] = ei.astype(BF16)
            mas[a, 0, 128:256, :] = (-ei).astype(BF16)
    E = dict(
        s_f=start([f_cp]), w_f=wait([f_cp]), s_ma=start(e_cp), w_ma=gen_ma,
        s_w=start(w_cp + wn_cp), w_w=wait(w_cp[:16] + wn_cp), w_w2=wait(w_cp[16:]), s_g=start([g_cp]), w_g=wait([g_cp]),
        s_c=start(c_cp), w_c=wait(c_cp), s_x=start(x_cp), w_x=wait(x_cp),
        s_w0=start(w_cps(0, 0)), w_w0=wait(w_cps(0, 0)), s_w1=start(w_cps(1, 1)), s_wo=start(wo_cp),
        zero=zero_init)
    for m in range(8):
        E['s_bx%d' % m] = start([bx_cp[m]]); E['w_bx%d' % m] = wait([bx_cp[m]])

    begin_scope('B')

    def run_item(item):
        if isinstance(item, tuple) and item[0] == 'blk':
            @pl.when(R.z0 == 0)
            def _():
                for it in item[1]: run_item(it)
        elif isinstance(item, str):
            if item.startswith('scope:'):
                end_scope(); begin_scope(item[6:])
            else:
                E[item]()
        elif item[0] == 'p1': p1(item[1])()
        elif item[0] == 'p2': p2(*item[1:])()
        elif item[0] == 'mid': mid(item[1])()
        elif item[0] == 'p3': p3(*item[1:])()
        elif item[0] == 'p4': p4(item[1])()
        elif item[0] == 'proj': proj0[item[1]]()
        else: raise ValueError(item)
    for item in border(UR): run_item(item)
    end_scope()
    if not doA:
        for d_ in b_out: d_.wait()
        return

    begin_scope('HEADS')

    def pair(p, wcur, wnext, last):
        for tag, f in attention_steps(qi, ki, vi, ctx, 0, 2 * p, bq, bk): f()
        for f in proj_steps(1, 1, xi, ci, wc, wcur, qb, kb, vb, rc): f()
        for tag, f in attention_steps(qi, ki, vi, ctx, 1, 2 * p + 1, bq, bk): f()
        if not last:
            for f in proj_steps(0, 0, xi, ci, wc, wnext, qb, kb, vb, rc): f()

    def body(p, _):
        wcur = lax.rem(p, 3); wnext = lax.rem(p + 1, 3)
        for d in w_cps(p + 1, wnext): d.wait()
        for d in w_cps(jnp.minimum(p + 2, H // 2 - 1), lax.rem(p + 2, 3)): d.start()
        pair(p, wcur, wnext, False)
        return 0
    lax.fori_loop(0, H // 2 - 1, body, 0)
    for d in w_cps(0, (H // 2) % 3): d.wait()
    end_scope()
    begin_scope('LAST')
    pair(H // 2 - 1, (H // 2 - 1) % 3, 0, True)

    end_scope()
    begin_scope('OUT')
    for d in wo_cp: d.wait()
    for d_ in b_out: d_.wait()
    ctxi = ctx.bitcast(jnp.int32); woi = wos.bitcast(jnp.int32)

    def a_out_cps(r16, osl):
        return [cp(ost.at[osl, a], out_hbm.at[pl.ds(r16, RO // 16), :, pl.ds(a * 128, 128)], osem.at[8 + osl * 8 + a]) for a in range(8)]

    def obody(r, _):
        r0 = r * (RO // 16); h0 = pl.multiple_of(r * (RO // 2), RO // 2)
        osl = r & 1

        @pl.when(r >= 2)
        def _():
            for d_ in a_out_cps(r0 - 2 * (RO // 16), osl): d_.wait()
        lhs = jnp.concatenate([bf(ctxi[hh, pl.ds(h0, RO // 2), :]) for hh in range(H)], axis=1)
        rhs = jnp.concatenate([bf(woi[a]) for a in range(8)], axis=1)
        o = jnp.dot(lhs, rhs, preferred_element_type=F32)
        for a in range(8):
            ost[osl, a] = o[:, a * 128:(a + 1) * 128].astype(BF16).reshape(RO // 16, 16, 128)
        for d_ in a_out_cps(r0, osl): d_.start()
        return 0
    lax.fori_loop(0, S // RO, obody, 0)
    for r in (S // RO - 2, S // RO - 1):
        for d_ in a_out_cps(r * (RO // 16), r & 1): d_.wait()
    end_scope()


def inter(*lists):
    lists = [l for l in lists if l]; it = []
    for li, l in enumerate(lists):
        for k, x in enumerate(l): it.append(((k + 0.5) / len(l), li, x))
    it.sort(key=lambda t: (t[0], t[1]))
    return [x for _, _, x in it]


def timed_border(mid_rate=130.0, mid_start=6200, p4proj=True):
    def border(UR):
        o = ['s_ma', 's_f'] + ['s_bx%d' % m for m in range(8)] + ['s_w', 'zero', 'w_ma', 'w_f']
        for m in range(8):
            o += ['w_bx%d' % m, ('p1', 2 * m), ('p1', 2 * m + 1)]
        o += ['scope:P2']
        items = []; t = 0.0
        for tt in range(4):
            for a in range(16): items.append((t, ('p2', a, tt * 128, (tt + 1) * 128))); t += 128
        for a in range(16): items.append((t, ('p2', a, 512, 528))); t += 20
        tm = mid_start; last = {}
        for k0 in range(0, 528, UR):
            items.append((tm, ('mid', k0))); last[k0 // 128] = tm; tm += mid_rate * UR / 8
        for tt in range(5):
            t = max(t, last[tt] + 1)
            for a in range(16): items.append((t, ('p3', a, tt))); t += 128
        items.sort(key=lambda x: x[0])
        seq = [x for _, x in items]; pos = {x: i for i, x in enumerate(seq)}
        for x in seq:
            if x[0] == 'mid': assert pos[x] > max(pos[y] for y in seq if y[0] == 'p2' and y[2] == x[1] // 128 * 128)
            if x[0] == 'p3': assert pos[x] > max(pos[y] for y in seq if y[0] == 'mid' and y[1] // 128 == x[2])
        for _, x in items:
            if x == ('mid', 0): o += ['scope:WW', 'w_w', 's_g', 's_c', 's_w0', 's_x', 'w_w2', 'scope:S']
            o.append(x)
        o += ['scope:WX', 'w_g', 'w_c', 'w_w0', 'w_x', 's_w1', 's_wo', 'scope:P4']
        proj = [('proj', i) for i in range(16)]
        if p4proj: o += inter([('p4', a) for a in range(16)], proj)
        else: o += [('p4', a) for a in range(16)] + proj
        return o
    return border


def border_base(UR):
    o = ['s_f'] + ['s_bx%d' % m for m in range(8)] + ['s_ma', 's_w', 's_g', 's_c', 's_x', 's_w0', 'zero', 'w_f']
    for m in range(8):
        o += ['w_bx%d' % m, ('p1', 2 * m), ('p1', 2 * m + 1)]
    o += ['scope:P2', 'w_ma'] + [('p2', a, 0, 528) for a in range(16)]
    o += ['scope:MID', 'w_w'] + [('mid', k0) for k0 in range(0, 528, UR)]
    o += ['scope:P3'] + [('p3', a, t) for a in range(16) for t in range(5)]
    o += ['scope:P4', 'w_g'] + [('p4', a) for a in range(16)]
    o += ['scope:PROJ0', 'w_c', 'w_x', 'w_w0', 's_w1', 's_wo'] + [('proj', i) for i in range(16)]
    return o


def make_fn(scopes=False, UR=8, bq=256, bk=512, rc=256, RO=256, border=None, tdtype=BF16, doA=True):
    global SCOPES
    SCOPES = scopes
    FTb, Gb, F128, TW = _consts()
    if border is None: border = timed_border()

    def fn(A_x, A_c_kv, A_w_q, A_w_uk, A_w_uv, A_w_o, B_x, B_w_r, B_w_i):
        x = A_x.reshape(S, M); c = A_c_kv.reshape(S, C); wo = A_w_o.reshape(H * D, M)
        bx = B_x.reshape(128, 16, DM)
        out = pl.pallas_call(
            functools.partial(kernel, UR=UR, bq=bq, bk=bk, rc=rc, RO=RO, border=border, doA=doA),
            in_specs=[pl.BlockSpec(memory_space=pltpu.SMEM)] + [pl.BlockSpec(memory_space=pl.ANY)] * 13,
            out_specs=pl.BlockSpec(memory_space=pl.ANY),
            out_shape=jax.ShapeDtypeStruct((128, 16, M + DM), BF16),
            scratch_shapes=[
                pltpu.VMEM((M // 128, S, 128), BF16),
                pltpu.VMEM((C // 128, S, 128), BF16),
                pltpu.VMEM((3, M + 2 * C, D), jnp.uint32),
                pltpu.VMEM((2, S, D), BF16), pltpu.VMEM((2, S, D), BF16), pltpu.VMEM((2, S, D), BF16),
                pltpu.VMEM((H, S, D), BF16),
                pltpu.VMEM((8, H * D, 128), BF16),
                pltpu.VMEM((8, 128, DM), jnp.uint32),
                pltpu.VMEM((16, 256, 128), jnp.uint32), pltpu.VMEM((16, 256, 128), jnp.uint32),
                pltpu.VMEM((2, 1, S), BF16),
                pltpu.VMEM((16, 528, 128), BF16), pltpu.VMEM((16, 528, 128), BF16),
                [pltpu.VMEM((4, 16, 128, 128), F32) for t in range(5)],
                pltpu.VMEM((16, 128, 640), F32), pltpu.VMEM((16, 128, 512), F32),
                pltpu.VMEM((4, 2, 272, 128), BF16), pltpu.VMEM((4, 2, 256, 128), BF16),
                pltpu.VMEM((16, 2, 256, 128), BF16),
                pltpu.VMEM((2, 128, 128), F32), pltpu.VMEM((32, 128), F32),
                pltpu.VMEM((2, 8, RO // 16, 16, 128), BF16),
                pltpu.SemaphoreType.DMA((68,)), pltpu.SemaphoreType.DMA((3, 3)), pltpu.SemaphoreType.DMA((24,)),
            ],
            compiler_params=pltpu.CompilerParams(vmem_limit_bytes=126 * 2 ** 20),
        )(jnp.zeros((1,), jnp.int32), x, c, A_w_q, A_w_uk, A_w_uv, wo, bx, B_w_r.T, B_w_i.T,
          jnp.asarray(FTb), jnp.asarray(Gb), jnp.asarray(F128), jnp.asarray(TW))
        return out.reshape(1, S, M + DM)
    return fn


_fn = make_fn()


@jax.jit
def pallas_concat_heads__compressed_kv_cla__spectral_gfnet__prompt_kernel(
    A_x: jax.Array,
    A_c_kv: jax.Array,
    A_w_q: jax.Array,
    A_w_uk: jax.Array,
    A_w_uv: jax.Array,
    A_w_o: jax.Array,
    B_x: jax.Array,
    B_w_r: jax.Array,
    B_w_i: jax.Array,
):
    return _fn(A_x, A_c_kv, A_w_q, A_w_uk, A_w_uv, A_w_o, B_x, B_w_r, B_w_i)
```

```python
import functools
import numpy as np
import jax
import jax.numpy as jnp
from jax import lax
from jax.experimental import pallas as pl
from jax.experimental.pallas import tpu as pltpu

S = 2048; D = 128; H = 32; M = 1024; C = 512; DM = 1024
NT = (((1,), (1,)), ((), ()))
NEG = -1e30
LOG2E = 1.4426950408889634
F32 = jnp.float32; BF16 = jnp.bfloat16


def bf(x): return pltpu.bitcast(x, BF16)

def _kset(j):
    cA, cB = (0, 4) if j == 0 else (j, 8 - j)
    e = np.arange(64)
    return np.concatenate([cA + 8 * e, cB + 8 * e])


def _bf16_np(a):
    import ml_dtypes
    return np.asarray(a, dtype=np.float32).astype(ml_dtypes.bfloat16)


def _consts():
    b = np.arange(128); alt = (-1.0) ** b
    FT = np.zeros((4, 272, 256)); G = np.zeros((4, 256, 256))
    for j in range(4):
        k = _kset(j)
        th = 2 * np.pi * np.outer(k, b) / 1024
        cw = (np.where(k == 0, 1.0, 2.0) / 1024)[:, None]
        if j == 0:
            A = (k % 8 == 0)[:, None]
            FT[0, :128, :128] = np.where(A, np.cos(th), 0); FT[0, :128, 128:] = np.where(~A, np.cos(th), 0)
            FT[0, 128:256, :128] = np.where(A, -np.sin(th), 0); FT[0, 128:256, 128:] = np.where(~A, -np.sin(th), 0)
            FT[0, 256, :128] = alt
            G[0, :128, :128] = np.where(A, cw * np.cos(th), 0); G[0, 128:, :128] = np.where(A, -cw * np.sin(th), 0)
            G[0, :128, 128:] = np.where(~A, cw * np.cos(th), 0); G[0, 128:, 128:] = np.where(~A, -cw * np.sin(th), 0)
            G[0, 128, :128] = alt / 1024
        else:
            s = np.where(k % 8 == j, 1.0, -1.0)[:, None]
            FT[j, :128, :128] = np.cos(th); FT[j, :128, 128:] = s * np.sin(th)
            FT[j, 128:256, :128] = -np.sin(th); FT[j, 128:256, 128:] = s * np.cos(th)
            G[j, :128, :128] = cw * np.cos(th); G[j, 128:, :128] = -cw * np.sin(th)
            G[j, :128, 128:] = s * cw * np.sin(th); G[j, 128:, 128:] = s * cw * np.cos(th)
    G = G / 2048
    E = np.exp(-2j * np.pi * np.outer(b, b) / 128)
    F128 = np.stack([E.real, E.imag]).astype(np.float32)
    TW = np.exp(-2j * np.pi * np.outer(np.arange(16), b) / 2048)
    TW = np.concatenate([TW.real, TW.imag]).astype(np.float32)
    FTb = FT.reshape(4, 272, 2, 128).transpose(0, 2, 1, 3)
    Gb = G.reshape(4, 256, 2, 128).transpose(0, 2, 1, 3)
    return _bf16_np(FTb), _bf16_np(Gb), F128, TW


def _r4(x0, x1, x2, x3, inverse):
    t0 = (x0[0] + x2[0], x0[1] + x2[1]); t1 = (x0[0] - x2[0], x0[1] - x2[1])
    t2 = (x1[0] + x3[0], x1[1] + x3[1]); t3 = (x1[0] - x3[0], x1[1] - x3[1])
    y0 = (t0[0] + t2[0], t0[1] + t2[1]); y2 = (t0[0] - t2[0], t0[1] - t2[1])
    a = (t1[0] + t3[1], t1[1] - t3[0])
    b = (t1[0] - t3[1], t1[1] + t3[0])
    return (y0, b, y2, a) if inverse else (y0, a, y2, b)


def _tw(x, m, inverse):
    m = m % 16
    if m == 0: return x
    xr, xi = x
    sg = -1.0 if inverse else 1.0
    if m == 4:
        return (xi, -xr) if not inverse else (-xi, xr)
    r = float(np.sqrt(0.5))
    if m == 2:
        if not inverse: return ((xr + xi) * r, (xi - xr) * r)
        return ((xr - xi) * r, (xi + xr) * r)
    if m == 6:
        if not inverse: return ((xi - xr) * r, (xr + xi) * (-r))
        return ((xr + xi) * (-r), (xr - xi) * r)
    c = float(np.cos(2 * np.pi * m / 16)); s = float(np.sin(2 * np.pi * m / 16)) * sg
    return (xr * c + xi * s, xi * c - xr * s)


def fft16(xs, inverse):
    A = [None] * 4
    for n2 in range(4):
        ys = _r4(xs[n2], xs[4 + n2], xs[8 + n2], xs[12 + n2], inverse)
        A[n2] = [_tw(ys[k1], n2 * k1, inverse) for k1 in range(4)]
    out = [None] * 16
    for k1 in range(4):
        ys = _r4(A[0][k1], A[1][k1], A[2][k1], A[3][k1], inverse)
        for k2 in range(4):
            out[k1 + 4 * k2] = ys[k2]
    return out


def attention_steps(qi, ki, vi, ctx, slot, h, bq, bk):
    def ld(ref, r0, r1): return bf(ref[slot, r0 // 2:r1 // 2, :])
    nq = S // bq

    def tiles(i):
        out = []; k0 = 0
        while k0 < i * bq:
            k1 = min(k0 + bk, i * bq); out.append((k0, k1, 0)); k0 = k1
        for t in range(bq // 128):
            out.append((i * bq + t * 128, i * bq + (t + 1) * 128, t * 128))
        return out
    state = {'ms': None, 'sl': []}
    sts = {}
    steps = []

    def qk(i, tile):
        def f():
            k0, k1, r0 = tile
            s = lax.dot_general(ld(qi, i * bq + r0, (i + 1) * bq), ld(ki, k0, k1), NT, preferred_element_type=F32)
            if k1 > i * bq:
                row = lax.broadcasted_iota(jnp.int32, (128, 128), 0)
                col = lax.broadcasted_iota(jnp.int32, (128, 128), 1)
                top = jnp.where(col <= row, s[:128], NEG)
                s = jnp.concatenate([top, s[128:]], axis=0) if s.shape[0] > 128 else top
            state['sl'].append(s)
            mx = s[:, :128]
            for c in range(1, (k1 - k0) // 128):
                mx = jnp.maximum(mx, s[:, c * 128:(c + 1) * 128])
            ms = state['ms']
            if ms is None: state['ms'] = mx
            elif r0 == 0: state['ms'] = jnp.maximum(ms, mx)
            else: state['ms'] = jnp.concatenate([ms[:r0], jnp.maximum(ms[r0:], mx)], axis=0)
        return f

    def begin(i):
        def f():
            sts[i] = {'m': jnp.max(state['ms'], axis=1, keepdims=True), 'l': None, 'acc': None, 's': state['sl']}
            state['sl'] = []; state['ms'] = None
        return f

    def pv(i, tile, j):
        def f():
            st = sts[i]; s = st['s'][j]
            k0, k1, r0 = tile
            p = jnp.exp2(s - st['m'][r0:])
            ls = jnp.sum(p, axis=1, keepdims=True)
            o = jnp.dot(p.astype(BF16), ld(vi, k0, k1), preferred_element_type=F32)
            if st['l'] is None: st['l'] = ls; st['acc'] = o
            elif r0 == 0: st['l'] = st['l'] + ls; st['acc'] = st['acc'] + o
            else:
                st['l'] = jnp.concatenate([st['l'][:r0], st['l'][r0:] + ls], axis=0)
                st['acc'] = jnp.concatenate([st['acc'][:r0], st['acc'][r0:] + o], axis=0)
        return f

    def fin(i):
        def f():
            st = sts[i]
            l = st['l']
            r = pltpu.reciprocal(l, approx=True); r = r * (2.0 - l * r)
            ctx[h, i * bq:(i + 1) * bq, :] = (st['acc'] * r).astype(BF16)
        return f
    for t in tiles(0): steps.append((('qk', 0), qk(0, t)))
    for i in range(nq):
        steps.append((('begin', i), begin(i)))
        tn = tiles(i + 1) if i + 1 < nq else []; tc = tiles(i)
        for j in range(max(len(tn), len(tc))):
            if j < len(tn): steps.append((('qk', i + 1), qk(i + 1, tn[j])))
            if j < len(tc): steps.append((('pv', i, j), pv(i, tc[j], j)))
        steps.append((('fin', i), fin(i)))
    return steps


def proj_steps(par, slot, xi, ci, wc, wslot, qb, kb, vb, rc):
    def half(w32):
        w = (w32 << 16) if par == 0 else (w32 & jnp.uint32(0xffff0000))
        return pltpu.bitcast(w, F32).astype(BF16)
    st = {}
    steps = []

    def getw():
        if 'wq' not in st:
            st['wq'] = half(wc[wslot, 0:M, :])
            st['wkv'] = jnp.concatenate([half(wc[wslot, M:M + C, :]), half(wc[wslot, M + C:, :])], axis=1)

    def qchunk(r):
        def f():
            getw()
            lhs = jnp.concatenate([bf(xi[j, r * rc // 2:(r + 1) * rc // 2, :]) for j in range(M // 128)], axis=1)
            q = jnp.dot(lhs, st['wq'], preferred_element_type=F32) * (D ** -0.5 * LOG2E)
            qb[slot, r * rc:(r + 1) * rc, :] = q.astype(BF16)
        return f

    def kvchunk(r):
        def f():
            getw()
            lhs = jnp.concatenate([bf(ci[j, r * rc // 2:(r + 1) * rc // 2, :]) for j in range(C // 128)], axis=1)
            kv = jnp.dot(lhs, st['wkv'], preferred_element_type=F32)
            kb[slot, r * rc:(r + 1) * rc, :] = kv[:, :D].astype(BF16)
            vb[slot, r * rc:(r + 1) * rc, :] = kv[:, D:].astype(BF16)
        return f
    for r in range(S // rc):
        steps.append(kvchunk(r)); steps.append(qchunk(r))
    return steps


SCOPES = False
DYN_A = tuple(range(8, 16))
OUT_INLINE = False
_stack = []
def begin_scope(n):
    if SCOPES:
        sc = jax.named_scope(n); sc.__enter__(); _stack.append(sc)
def end_scope():
    if SCOPES:
        _stack.pop().__exit__(None, None, None)


def b_steps(R, UR):
    r2 = float(np.sqrt(0.5))
    HI = jnp.uint32(0xffff0000)
    fi = R.fs.bitcast(jnp.int32); gi = R.gs.bitcast(jnp.int32); mai = R.mas.bitcast(jnp.int32)
    x1ri = R.x1r.bitcast(jnp.int32); x1ii = R.x1i.bitcast(jnp.int32)

    def p1(a):
        m, par = a // 2, a % 2

        def f():
            xa = []
            for A in range(8):
                w = R.bxs[m, :, A * 128:(A + 1) * 128]
                xa.append(pltpu.bitcast(w << 16 if par == 0 else w & HI, F32))
            u0, u1 = xa[0] + xa[4], xa[0] - xa[4]; u2, u3 = xa[2] + xa[6], xa[2] - xa[6]
            u4, u5 = xa[1] + xa[5], xa[1] - xa[5]; u6, u7 = xa[3] + xa[7], xa[3] - xa[7]
            s_, t_ = u0 + u2, u4 + u6
            d57, s57 = (u5 - u7) * r2, (u5 + u7) * r2
            L = [(s_ + t_, s_ - t_), (u1 + d57, (u3 + s57) * -1.0), (u0 - u2, u6 - u4), (u1 - d57, u3 - s57)]
            for j in range(4):
                data = jnp.concatenate(L[j], axis=1).astype(BF16)
                nr = 272 if j == 0 else 256
                lhs = jnp.concatenate([bf(fi[j, 0, 0:nr // 2, :]), bf(fi[j, 1, 0:nr // 2, :])], axis=1)
                o = lax.dot_general(lhs, data, NT, preferred_element_type=F32).astype(BF16)
                R.x1r[a, j * 128:(j + 1) * 128, :] = o[:128]
                R.x1i[a, j * 128:(j + 1) * 128, :] = o[128:256]
                if j == 0:
                    R.x1r[a, 512:528, :] = o[256:272]
        return f

    def p2(a, k0, k1):
        def f():
            lhs = jnp.concatenate([bf(x1ri[a, k0 // 2:k1 // 2, :]), bf(x1ii[a, k0 // 2:k1 // 2, :])], axis=1)
            rhs = jnp.concatenate([bf(mai[a, 0]), bf(mai[a, 1])], axis=1)
            o = jnp.dot(lhs, rhs, preferred_element_type=F32)
            for t in range(k0 // 128, (k1 + 127) // 128):
                l0 = max(k0, t * 128); l1 = min(k1, (t + 1) * 128)
                R.vt[t][0, a, l0 - t * 128:l1 - t * 128, :] = o[l0 - k0:l1 - k0, :128]
                R.vt[t][1, a, l0 - t * 128:l1 - t * 128, :] = o[l0 - k0:l1 - k0, 128:]
        return f

    def mid(k0):
        if True:
            j, rem = k0 // 128, k0 % 128
            hf, e0 = rem // 64, rem % 64
            c = (0, 4)[hf] if j == 0 else (j, 8 - j)[hf]

            def wload(cc):
                wr_ = R.wr32[cc, pl.ds(c // 2 + 4 * e0, UR, stride=4), :]
                wi_ = R.wi32[cc, pl.ds(c // 2 + 4 * e0, UR, stride=4), :]
                if c % 2 == 0:
                    return pltpu.bitcast(wr_ << 16, F32), pltpu.bitcast(wi_ << 16, F32)
                return pltpu.bitcast(wr_ & HI, F32), pltpu.bitcast(wi_ & HI, F32)
        def cmul(x, w):
            return (x[0] * w[0] - x[1] * w[1], x[0] * w[1] + x[1] * w[0])

        def f():
            t, kk = k0 // 128, k0 % 128
            xs_ = [((R.vt[t][R.z0, a, kk:kk + UR, :], R.vt[t][R.z0 + 1, a, kk:kk + UR, :]) if a in DYN_A else
                    (R.vt[t][0, a, kk:kk + UR, :], R.vt[t][1, a, kk:kk + UR, :])) for a in range(16)]
            X = fft16(xs_, False)
            Y = [cmul(X[cc], wload(cc)) for cc in range(16)]
            if k0 == 0:
                xn = [(R.vt[4][0, a, 0:UR, :], R.vt[4][1, a, 0:UR, :]) for a in range(16)]
                XN = fft16(xn, False)
                YN = [cmul(XN[cc], (jnp.broadcast_to(R.wn[0, :, cc * 128:(cc + 1) * 128].astype(F32), (UR, 128)),
                                    jnp.broadcast_to(R.wn[1, :, cc * 128:(cc + 1) * 128].astype(F32), (UR, 128))))
                      for cc in range(16)]
                ln = lax.broadcasted_iota(jnp.int32, (UR, 128), 1)
                rw = lax.broadcasted_iota(jnp.int32, (UR, 128), 0)
                idx = (128 - ln) & 127
                Pm = [(jnp.take_along_axis(Y[c][0] + YN[c][1], idx, axis=1),
                       jnp.take_along_axis(Y[c][1] - YN[c][0], idx, axis=1)) for c in range(16)]
                Y2 = []
                for cc in range(16):
                    fr_ = jnp.where(ln == 0, Pm[(16 - cc) % 16][0], Pm[15 - cc][0])
                    fi2 = jnp.where(ln == 0, Pm[(16 - cc) % 16][1], Pm[15 - cc][1])
                    tr_ = (Y[cc][0] - YN[cc][1] + fr_) * 0.5
                    ti_ = (Y[cc][1] + YN[cc][0] - fi2) * 0.5
                    Y2.append((jnp.where(rw == 0, tr_, Y[cc][0]), jnp.where(rw == 0, ti_, Y[cc][1])))
                Y = Y2
            Tt = fft16(Y, True)
            for a in range(16):
                R.vt[t][2, a, kk:kk + UR, :] = Tt[a][0]
                R.vt[t][3, a, kk:kk + UR, :] = Tt[a][1]
        return f

    def p3(a, t):
        def f():
            lhs = jnp.concatenate([bf(mai[a, 0]), bf(mai[a, 1])], axis=1)
            data = jnp.concatenate([R.vt[t][2, a], R.vt[t][3, a]], axis=1).astype(BF16)
            o = lax.dot_general(lhs, data, NT, preferred_element_type=F32)
            R.y1r[a, :, t * 128:(t + 1) * 128] = o[:128]
            R.y1i[a, :, t * 128:(t + 1) * 128] = o[128:]
        return f

    lane = lax.broadcasted_iota(jnp.int32, (128, 128), 1)
    st = {}

    def p4(a):
        def f():
            U = []
            for j in range(4):
                yr = R.y1r[a, :, j * 128:(j + 1) * 128]; yi = R.y1i[a, :, j * 128:(j + 1) * 128]
                lhs = jnp.concatenate([yr, yi], axis=1).astype(BF16)
                rhs = jnp.concatenate([bf(gi[j, 0]), bf(gi[j, 1])], axis=1)
                o = jnp.dot(lhs, rhs, preferred_element_type=F32)
                U.append((o[:, :128], o[:, 128:]))
            T0, T4 = U[0]; U1r, U1i = U[1]; U2r, U2i = U[2]; U3r, U3i = U[3]
            P, Q = T0 + T4, T0 - T4
            A_, B_ = P + U2r, P - U2r
            s13 = U1r + U3r; d = U3i - U1i
            Qm, Qp = Q - U2i, Q + U2i
            t1, t2 = U1r - U3r, U1i + U3i
            e1, e3 = (t1 - t2) * r2, (t1 + t2) * r2
            st[a] = [A_ + s13, Qm + e1, B_ + d, Qp - e3, A_ - s13, Qm - e1, B_ - d, Qp + e3]
            if a % 2 == 1:
                m = a // 2
                for A in range(8):
                    R.bxs[m, :, A * 128:(A + 1) * 128] = pltpu.bitcast(
                        pltpu.pack_elementwise([st[a - 1][A], st[a][A]], packed_dtype=BF16), jnp.uint32)
                if R.out_inline: R.b_out[m].start()
        return f
    return p1, p2, mid, p3, p4


class NS:
    pass


def kernel(z_ref, x_hbm, c_hbm, wq_hbm, wk_hbm, wv_hbm, wo_hbm, bx_hbm, wr_hbm, wi_hbm, f_hbm, g_hbm, e_hbm, tw_hbm,
           out_hbm,
           xs, cs, wc, qb, kb, vb, ctx, wos, bxs, wr32, wi32, wn, x1r, x1i, vt, y1r, y1i,
           fs, gs, mas, es, tws, ost,
           sem, wsem, osem, *, UR, bq, bk, rc, RO, border, doA=True):
    def cp(src, dst, s): return pltpu.make_async_copy(src, dst, s)
    bx_u = bx_hbm.bitcast(jnp.uint32)
    bx_cp = [cp(bx_u.at[:, m, :], bxs.at[m], sem.at[m]) for m in range(8)]
    f_cp = cp(f_hbm, fs, sem.at[8])
    e_cp = [cp(e_hbm, es, sem.at[9]), cp(tw_hbm, tws, sem.at[10])]
    g_cp = cp(g_hbm, gs, sem.at[11])
    wr_u = wr_hbm.at[pl.ds(0, 512), :].bitcast(jnp.uint32)
    wi_u = wi_hbm.at[pl.ds(0, 512), :].bitcast(jnp.uint32)
    w_cp = [cp(wr_u.at[:, cc * 128:(cc + 1) * 128], wr32.at[cc], sem.at[36 + cc]) for cc in range(16)]
    w_cp += [cp(wi_u.at[:, cc * 128:(cc + 1) * 128], wi32.at[cc], sem.at[52 + cc]) for cc in range(16)]
    wn_cp = [cp(wr_hbm.at[pl.ds(512, 1), :], wn.at[0], sem.at[12]), cp(wi_hbm.at[pl.ds(512, 1), :], wn.at[1], sem.at[13])]
    x_cp = [cp(x_hbm.at[:, a * 128:(a + 1) * 128], xs.at[a], sem.at[14 + a]) for a in range(8)]
    c_cp = [cp(c_hbm.at[:, a * 128:(a + 1) * 128], cs.at[a], sem.at[22 + a]) for a in range(4)]
    wo_cp = [cp(wo_hbm.at[:, a * 128:(a + 1) * 128], wos.at[a], sem.at[26 + a]) for a in range(8)]
    wq_u = wq_hbm.bitcast(jnp.uint32); wk_u = wk_hbm.bitcast(jnp.uint32); wv_u = wv_hbm.bitcast(jnp.uint32)
    out_u = out_hbm.bitcast(jnp.uint32)
    b_out = [cp(bxs.at[m], out_u.at[:, m, pl.ds(DM, DM)], osem.at[m]) for m in range(8)]

    def w_cps(j, wslot):
        return [cp(wq_u.at[:, j, :], wc.at[wslot, pl.ds(0, M), :], wsem.at[wslot, 0]),
                cp(wk_u.at[:, j, :], wc.at[wslot, pl.ds(M, C), :], wsem.at[wslot, 1]),
                cp(wv_u.at[:, j, :], wc.at[wslot, pl.ds(M + C, C), :], wsem.at[wslot, 2])]
    R = NS()
    R.z0 = z_ref[0]
    R.out_inline = OUT_INLINE
    R.fs, R.gs, R.mas, R.x1r, R.x1i, R.vt = fs, gs, mas, x1r, x1i, vt
    R.bxs, R.wr32, R.wi32, R.wn, R.y1r, R.y1i, R.b_out = bxs, wr32, wi32, wn, y1r, y1i, b_out
    p1, p2, mid, p3, p4 = b_steps(R, UR)

    xi = xs.bitcast(jnp.int32); ci = cs.bitcast(jnp.int32)
    qi = qb.bitcast(jnp.int32); ki = kb.bitcast(jnp.int32); vi = vb.bitcast(jnp.int32)
    proj0 = proj_steps(0, 0, xi, ci, wc, 0, qb, kb, vb, rc)

    def start(ds): return lambda: [d.start() for d in ds]
    def wait(ds): return lambda: [d.wait() for d in ds]

    def zero_init():
        for a in range(16):
            x1i[a, pl.ds(512, 16), :] = jnp.zeros((16, 128), BF16)
    def gen_ma():
        for d in e_cp: d.wait()
        fr = es[0]; fi_ = es[1]
        for a in range(16):
            tr_ = jnp.broadcast_to(tws[a:a + 1, :], (128, 128)); ti_ = jnp.broadcast_to(tws[16 + a:17 + a, :], (128, 128))
            er = fr * tr_ - fi_ * ti_
            ei = fr * ti_ + fi_ * tr_
            erb = er.astype(BF16)
            mas[a, 0, 0:128, :] = erb
            mas[a, 1, 128:256, :] = erb
            mas[a, 1, 0:128, :] = ei.astype(BF16)
            mas[a, 0, 128:256, :] = (-ei).astype(BF16)
    E = dict(
        s_f=start([f_cp]), w_f=wait([f_cp]), s_ma=start(e_cp), w_ma=gen_ma,
        s_w=start(w_cp + wn_cp), s_wr=start(w_cp[:16] + wn_cp), s_wi=start(w_cp[16:]), w_w=wait(w_cp[:16] + wn_cp), w_w2=wait(w_cp[16:]), s_g=start([g_cp]), w_g=wait([g_cp]),
        s_c=start(c_cp), w_c=wait(c_cp), s_x=start(x_cp), w_x=wait(x_cp),
        s_w0=start(w_cps(0, 0)), w_w0=wait(w_cps(0, 0)), s_w1=start(w_cps(1, 1)), s_wo=start(wo_cp),
        w_w1=wait(w_cps(1, 1)), w_wo=wait(wo_cp),
        zero=zero_init, s_out=start(b_out), s_out_a=start(b_out[:4]), s_out_b=start(b_out[4:]))
    for m in range(8):
        E['s_bx%d' % m] = start([bx_cp[m]]); E['w_bx%d' % m] = wait([bx_cp[m]])

    begin_scope('B')

    def run_item(item):
        if isinstance(item, tuple) and item[0] == 'blk':
            @pl.when(R.z0 == 0)
            def _():
                for it in item[1]: run_item(it)
        elif isinstance(item, str):
            if item.startswith('scope:'):
                end_scope(); begin_scope(item[6:])
            else:
                E[item]()
        elif item[0] == 'p1': p1(item[1])()
        elif item[0] == 'p2': p2(*item[1:])()
        elif item[0] == 'mid': mid(item[1])()
        elif item[0] == 'p3': p3(*item[1:])()
        elif item[0] == 'p4': p4(item[1])()
        elif item[0] == 'proj': proj0[item[1]]()
        else: raise ValueError(item)
    for item in border(UR): run_item(item)
    end_scope()
    if not doA:
        if doA is not None:
            for d_ in b_out: d_.wait()
        return

    begin_scope('HEADS')

    ctxi = ctx.bitcast(jnp.int32); woi = wos.bitcast(jnp.int32)

    def a_out_cps(r16, osl):
        return [cp(ost.at[osl, a], out_hbm.at[pl.ds(r16, RO // 16), :, pl.ds(a * 128, 128)], osem.at[8 + osl * 8 + a]) for a in range(8)]

    def out_pieces(r):
        def piece(a):
            def f():
                lhs = jnp.concatenate([bf(ctxi[hh, r * RO // 2:(r + 1) * RO // 2, :]) for hh in range(H)], axis=1)
                o = jnp.dot(lhs, bf(woi[a]), preferred_element_type=F32)
                ost[r & 1, a] = o.astype(BF16).reshape(RO // 16, 16, 128)
            return f
        return [piece(a) for a in range(8)]

    def head(slot, h, proj, fill_at=None):
        pi = 0
        for tag, f in attention_steps(qi, ki, vi, ctx, slot, h, bq, bk):
            f()
            if tag[0] == 'begin' and tag[1] in (fill_at or (0, S // bq - 1)) and pi < len(proj):
                proj[pi](); pi += 1
        for f in proj[pi:]: f()

    def pair(p, wcur, wnext, last):
        pr = proj_steps(1, 1, xi, ci, wc, wcur, qb, kb, vb, rc)
        head(0, 2 * p, pr[1::2] + pr[0::2])
        if last:
            head(1, 2 * p + 1, out_pieces(0), fill_at=(1, 2, S // bq - 1))
            for d_ in a_out_cps(0, 0): d_.start()
        else:
            pr = proj_steps(0, 0, xi, ci, wc, wnext, qb, kb, vb, rc)
            head(1, 2 * p + 1, pr[1::2] + pr[0::2])

    def body(p, _):
        wcur = lax.rem(p, 3); wnext = lax.rem(p + 1, 3)
        for d in w_cps(p + 1, wnext): d.wait()
        for d in w_cps(jnp.minimum(p + 2, H // 2 - 1), lax.rem(p + 2, 3)): d.start()
        pair(p, wcur, wnext, False)
        return 0
    lax.fori_loop(0, H // 2 - 1, body, 0)
    for d in w_cps(0, (H // 2) % 3): d.wait()
    for d in wo_cp: d.wait()
    end_scope()
    begin_scope('LAST')
    pair(H // 2 - 1, (H // 2 - 1) % 3, 0, True)

    end_scope()
    begin_scope('OUT')
    for d_ in b_out: d_.wait()
    def obody(r, _):
        r0 = r * (RO // 16); h0 = pl.multiple_of(r * (RO // 2), RO // 2)
        osl = r & 1

        @pl.when(r >= 2)
        def _():
            for d_ in a_out_cps(r0 - 2 * (RO // 16), osl): d_.wait()
        lhs = jnp.concatenate([bf(ctxi[hh, pl.ds(h0, RO // 2), :]) for hh in range(H)], axis=1)
        rhs = jnp.concatenate([bf(woi[a]) for a in range(8)], axis=1)
        o = jnp.dot(lhs, rhs, preferred_element_type=F32)
        for a in range(8):
            ost[osl, a] = o[:, a * 128:(a + 1) * 128].astype(BF16).reshape(RO // 16, 16, 128)
        for d_ in a_out_cps(r0, osl): d_.start()
        return 0
    lax.fori_loop(1, S // RO, obody, 0)
    for r in (S // RO - 2, S // RO - 1):
        for d_ in a_out_cps(r * (RO // 16), r & 1): d_.wait()
    end_scope()


def inter(*lists):
    lists = [l for l in lists if l]; it = []
    for li, l in enumerate(lists):
        for k, x in enumerate(l): it.append(((k + 0.5) / len(l), li, x))
    it.sort(key=lambda t: (t[0], t[1]))
    return [x for _, _, x in it]


def timed_border(mid_rate=130.0, mid_start=4500, p4proj=True, pmode=0):
    def border(UR):
        o = ['s_bx0', 's_ma', 's_f', 's_bx1', 's_bx2', 'zero', 'w_ma', 's_bx3', 'w_f']
        for m in range(8):
            o += ['w_bx%d' % m, ('p1', 2 * m), ('p1', 2 * m + 1)]
            if m == 0: o += ['s_bx4', 's_bx5']
            if m == 1: o += ['s_bx6', 's_bx7']
            if m == 2: o += ['s_wr']
            if m == 3: o += ['s_wi']
        o += ['scope:P2']
        items = []; t = 0.0
        for a in range(16): items.append((t, ('p2', a, 512, 528))); t += 20
        for tt in range(4):
            for a in range(16): items.append((t, ('p2', a, tt * 128, (tt + 1) * 128))); t += 128
        tm = mid_start; last = {}
        for k0 in range(0, 512, UR):
            items.append((tm, ('mid', k0))); last[k0 // 128] = tm; tm += mid_rate * UR / 8
        for tt in range(4):
            t = max(t, last[tt] + 1)
            for a in range(16): items.append((t, ('p3', a, tt))); t += 128
        items.sort(key=lambda x: x[0])
        seq = [x for _, x in items]; pos = {x: i for i, x in enumerate(seq)}
        for x in seq:
            if x[0] == 'mid': assert pos[x] > max(pos[y] for y in seq if y[0] == 'p2' and y[2] == x[1] // 128 * 128)
            if x[0] == 'p3': assert pos[x] > max(pos[y] for y in seq if y[0] == 'mid' and y[1] // 128 == x[2])
        for _, x in items:
            if x == ('mid', 0): o += ['scope:WW', 'w_w', 's_g', 's_c', 's_w0', 's_x', 'w_w2', 'scope:S']
            o.append(x)
        proj = [('proj', i) for i in range(16)]
        kv, qq = proj[0::2], proj[1::2]
        P4 = [('p4', a) for a in range(16)]
        if pmode == 0:
            o += ['scope:WX', 'w_g', 'w_c', 'w_w0', 'w_x', 's_w1', 's_wo', 'scope:P4']
            o += inter(P4, proj)
        elif pmode == 1:
            o += ['scope:WX', 'w_g', 'w_c', 'w_w0', 'w_x', 's_w1', 's_wo', 'scope:P4']
            o += inter(P4, kv) + qq
        elif pmode == 2:
            o += ['scope:WX', 'w_g', 'w_c', 'w_w0', 'w_x', 's_w1', 's_wo', 'scope:P4']
            o += inter(P4, qq) + kv
        elif pmode == 3:
            o += ['scope:WX', 'w_g', 'w_c', 'w_w0', 'w_x', 's_w1', 's_wo', 'scope:P4']
            o += inter(P4, qq + kv)
        elif pmode == 4:
            o += ['scope:WX', 'w_g', 'w_c', 'w_w0', 'w_x', 's_w1', 's_wo', 'scope:P4']
            o += proj[:2] + inter(P4, proj[2:])
        elif pmode == 5:
            o += ['scope:WX', 'w_g', 'w_c', 'w_w0', 'w_x', 's_w1', 's_wo', 'scope:P4']
            o += inter(P4, proj[:12]) + proj[12:]
        o += ['s_out']
        return o
    return border


def stage_border(blocks=True, first=3):
    def border(UR):
        o = ['s_bx0', 's_ma', 's_f', 's_bx1', 's_bx2', 'zero', 'w_ma', 's_bx3', 'w_f']
        for m in range(8):
            o += ['w_bx%d' % m, ('p1', 2 * m), ('p1', 2 * m + 1)]
            if m == 0: o += ['s_bx4', 's_bx5']
            if m == 1: o += ['s_bx6', 's_bx7']
            if m == 2: o += ['s_wr']
            if m == 3: o += ['s_wi']
        MID = lambda t: [('mid', k0) for k0 in range(t * 128, (t + 1) * 128, UR)]
        P3 = lambda t: [('p3', a, t) for a in range(16)]
        P2 = lambda t: [('p2', a, t * 128, (t + 1) * 128) for a in range(16)]
        P2n = [('p2', a, 512, 528) for a in range(16)]
        o += ['scope:P2'] + P2n + P2(0) + P2(1) + P2(2)
        o += ['scope:WW', 'w_w', 's_g', 's_c', 's_w0', 's_x', 'w_w2', 'scope:S']
        st = [inter(MID(0), P2(3)), inter(MID(1), P3(0)), inter(MID(2), P3(1)), inter(MID(3), P3(2)), P3(3)]
        for x in st:
            if blocks: o.append(('blk', x))
            else: o += x
        o += ['scope:WX', 'w_g', 'w_c', 'w_w0', 'w_x', 's_w1', 's_wo', 'scope:P4']
        o += inter([('p4', a) for a in range(16)], [('proj', i) for i in range(16)]) + ['s_out']
        return o
    return border


def make_fn(scopes=False, UR=8, bq=256, bk=512, rc=256, RO=256, border=None, tdtype=BF16, doA=True):
    global SCOPES
    SCOPES = scopes
    FTb, Gb, F128, TW = _consts()
    if border is None: border = timed_border()

    def fn(A_x, A_c_kv, A_w_q, A_w_uk, A_w_uv, A_w_o, B_x, B_w_r, B_w_i):
        x = A_x.reshape(S, M); c = A_c_kv.reshape(S, C); wo = A_w_o.reshape(H * D, M)
        bx = B_x.reshape(128, 16, DM)
        out = pl.pallas_call(
            functools.partial(kernel, UR=UR, bq=bq, bk=bk, rc=rc, RO=RO, border=border, doA=doA),
            in_specs=[pl.BlockSpec(memory_space=pltpu.SMEM)] + [pl.BlockSpec(memory_space=pl.ANY)] * 13,
            out_specs=pl.BlockSpec(memory_space=pl.ANY),
            out_shape=jax.ShapeDtypeStruct((128, 16, M + DM), BF16),
            scratch_shapes=[
                pltpu.VMEM((M // 128, S, 128), BF16),
                pltpu.VMEM((C // 128, S, 128), BF16),
                pltpu.VMEM((3, M + 2 * C, D), jnp.uint32),
                pltpu.VMEM((2, S, D), BF16), pltpu.VMEM((2, S, D), BF16), pltpu.VMEM((2, S, D), BF16),
                pltpu.VMEM((H, S, D), BF16),
                pltpu.VMEM((8, H * D, 128), BF16),
                pltpu.VMEM((8, 128, DM), jnp.uint32),
                pltpu.VMEM((16, 256, 128), jnp.uint32), pltpu.VMEM((16, 256, 128), jnp.uint32),
                pltpu.VMEM((2, 1, S), BF16),
                pltpu.VMEM((16, 528, 128), BF16), pltpu.VMEM((16, 528, 128), BF16),
                [pltpu.VMEM((4, 16, 128, 128), F32) for t in range(4)] + [pltpu.VMEM((2, 16, 16, 128), F32)],
                pltpu.VMEM((16, 128, 512), F32), pltpu.VMEM((16, 128, 512), F32),
                pltpu.VMEM((4, 2, 272, 128), BF16), pltpu.VMEM((4, 2, 256, 128), BF16),
                pltpu.VMEM((16, 2, 256, 128), BF16),
                pltpu.VMEM((2, 128, 128), F32), pltpu.VMEM((32, 128), F32),
                pltpu.VMEM((2, 8, RO // 16, 16, 128), BF16),
                pltpu.SemaphoreType.DMA((68,)), pltpu.SemaphoreType.DMA((3, 3)), pltpu.SemaphoreType.DMA((24,)),
            ],
            compiler_params=pltpu.CompilerParams(vmem_limit_bytes=126 * 2 ** 20),
        )(jnp.zeros((1,), jnp.int32), x, c, A_w_q, A_w_uk, A_w_uv, wo, bx, B_w_r.T, B_w_i.T,
          jnp.asarray(FTb), jnp.asarray(Gb), jnp.asarray(F128), jnp.asarray(TW))
        return out.reshape(1, S, M + DM)
    return fn


_fn = make_fn()


@jax.jit
def pallas_concat_heads__compressed_kv_cla__spectral_gfnet__prompt_kernel(
    A_x: jax.Array,
    A_c_kv: jax.Array,
    A_w_q: jax.Array,
    A_w_uk: jax.Array,
    A_w_uv: jax.Array,
    A_w_o: jax.Array,
    B_x: jax.Array,
    B_w_r: jax.Array,
    B_w_i: jax.Array,
):
    return _fn(A_x, A_c_kv, A_w_q, A_w_uk, A_w_uv, A_w_o, B_x, B_w_r, B_w_i)
```

```python
import functools
import numpy as np
import jax
import jax.numpy as jnp
from jax import lax
from jax.experimental import pallas as pl
from jax.experimental.pallas import tpu as pltpu

S = 2048; D = 128; H = 32; M = 1024; C = 512; DM = 1024
NT = (((1,), (1,)), ((), ()))
NEG = -1e30
LOG2E = 1.4426950408889634
F32 = jnp.float32; BF16 = jnp.bfloat16


def bf(x): return pltpu.bitcast(x, BF16)

def _kset(j):
    cA, cB = (0, 4) if j == 0 else (j, 8 - j)
    e = np.arange(64)
    return np.concatenate([cA + 8 * e, cB + 8 * e])


def _bf16_np(a):
    import ml_dtypes
    return np.asarray(a, dtype=np.float32).astype(ml_dtypes.bfloat16)


def _consts():
    b = np.arange(128); alt = (-1.0) ** b
    FT = np.zeros((4, 272, 256)); G = np.zeros((4, 256, 256))
    for j in range(4):
        k = _kset(j)
        th = 2 * np.pi * np.outer(k, b) / 1024
        cw = (np.where(k == 0, 1.0, 2.0) / 1024)[:, None]
        if j == 0:
            A = (k % 8 == 0)[:, None]
            FT[0, :128, :128] = np.where(A, np.cos(th), 0); FT[0, :128, 128:] = np.where(~A, np.cos(th), 0)
            FT[0, 128:256, :128] = np.where(A, -np.sin(th), 0); FT[0, 128:256, 128:] = np.where(~A, -np.sin(th), 0)
            FT[0, 256, :128] = alt
            G[0, :128, :128] = np.where(A, cw * np.cos(th), 0); G[0, 128:, :128] = np.where(A, -cw * np.sin(th), 0)
            G[0, :128, 128:] = np.where(~A, cw * np.cos(th), 0); G[0, 128:, 128:] = np.where(~A, -cw * np.sin(th), 0)
            G[0, 128, :128] = alt / 1024
        else:
            s = np.where(k % 8 == j, 1.0, -1.0)[:, None]
            FT[j, :128, :128] = np.cos(th); FT[j, :128, 128:] = s * np.sin(th)
            FT[j, 128:256, :128] = -np.sin(th); FT[j, 128:256, 128:] = s * np.cos(th)
            G[j, :128, :128] = cw * np.cos(th); G[j, 128:, :128] = -cw * np.sin(th)
            G[j, :128, 128:] = s * cw * np.sin(th); G[j, 128:, 128:] = s * cw * np.cos(th)
    G = G / 2048
    E = np.exp(-2j * np.pi * np.outer(b, b) / 128)
    F128 = np.stack([E.real, E.imag]).astype(np.float32)
    TW = np.exp(-2j * np.pi * np.outer(np.arange(16), b) / 2048)
    TW = np.concatenate([TW.real, TW.imag]).astype(np.float32)
    FTb = FT.reshape(4, 272, 2, 128).transpose(0, 2, 1, 3)
    Gb = G.reshape(4, 256, 2, 128).transpose(0, 2, 1, 3)
    return _bf16_np(FTb), _bf16_np(Gb), F128, TW


def _r4(x0, x1, x2, x3, inverse):
    t0 = (x0[0] + x2[0], x0[1] + x2[1]); t1 = (x0[0] - x2[0], x0[1] - x2[1])
    t2 = (x1[0] + x3[0], x1[1] + x3[1]); t3 = (x1[0] - x3[0], x1[1] - x3[1])
    y0 = (t0[0] + t2[0], t0[1] + t2[1]); y2 = (t0[0] - t2[0], t0[1] - t2[1])
    a = (t1[0] + t3[1], t1[1] - t3[0])
    b = (t1[0] - t3[1], t1[1] + t3[0])
    return (y0, b, y2, a) if inverse else (y0, a, y2, b)


def _tw(x, m, inverse):
    m = m % 16
    if m == 0: return x
    xr, xi = x
    sg = -1.0 if inverse else 1.0
    if m == 4:
        return (xi, -xr) if not inverse else (-xi, xr)
    r = float(np.sqrt(0.5))
    if m == 2:
        if not inverse: return ((xr + xi) * r, (xi - xr) * r)
        return ((xr - xi) * r, (xi + xr) * r)
    if m == 6:
        if not inverse: return ((xi - xr) * r, (xr + xi) * (-r))
        return ((xr + xi) * (-r), (xr - xi) * r)
    c = float(np.cos(2 * np.pi * m / 16)); s = float(np.sin(2 * np.pi * m / 16)) * sg
    return (xr * c + xi * s, xi * c - xr * s)


def fft16(xs, inverse):
    A = [None] * 4
    for n2 in range(4):
        ys = _r4(xs[n2], xs[4 + n2], xs[8 + n2], xs[12 + n2], inverse)
        A[n2] = [_tw(ys[k1], n2 * k1, inverse) for k1 in range(4)]
    out = [None] * 16
    for k1 in range(4):
        ys = _r4(A[0][k1], A[1][k1], A[2][k1], A[3][k1], inverse)
        for k2 in range(4):
            out[k1 + 4 * k2] = ys[k2]
    return out


def attention_steps(qi, ki, vi, ctx, slot, h, bq, bk):
    def ld(ref, r0, r1): return bf(ref[slot, r0 // 2:r1 // 2, :])
    nq = S // bq

    def tiles(i):
        out = []; k0 = 0
        while k0 < i * bq:
            k1 = min(k0 + bk, i * bq); out.append((k0, k1, 0)); k0 = k1
        for t in range(bq // 128):
            out.append((i * bq + t * 128, i * bq + (t + 1) * 128, t * 128))
        return out
    state = {'ms': None, 'sl': []}
    sts = {}
    steps = []

    def qk(i, tile):
        def f():
            k0, k1, r0 = tile
            s = lax.dot_general(ld(qi, i * bq + r0, (i + 1) * bq), ld(ki, k0, k1), NT, preferred_element_type=F32)
            if k1 > i * bq:
                row = lax.broadcasted_iota(jnp.int32, (128, 128), 0)
                col = lax.broadcasted_iota(jnp.int32, (128, 128), 1)
                top = jnp.where(col <= row, s[:128], NEG)
                s = jnp.concatenate([top, s[128:]], axis=0) if s.shape[0] > 128 else top
            state['sl'].append(s)
            mx = s[:, :128]
            for c in range(1, (k1 - k0) // 128):
                mx = jnp.maximum(mx, s[:, c * 128:(c + 1) * 128])
            ms = state['ms']
            if ms is None: state['ms'] = mx
            elif r0 == 0: state['ms'] = jnp.maximum(ms, mx)
            else: state['ms'] = jnp.concatenate([ms[:r0], jnp.maximum(ms[r0:], mx)], axis=0)
        return f

    def begin(i):
        def f():
            sts[i] = {'m': jnp.max(state['ms'], axis=1, keepdims=True), 'l': None, 'acc': None, 's': state['sl']}
            state['sl'] = []; state['ms'] = None
        return f

    def pv(i, tile, j):
        def f():
            st = sts[i]; s = st['s'][j]
            k0, k1, r0 = tile
            p = jnp.exp2(s - st['m'][r0:])
            ls = jnp.sum(p, axis=1, keepdims=True)
            o = jnp.dot(p.astype(BF16), ld(vi, k0, k1), preferred_element_type=F32)
            if st['l'] is None: st['l'] = ls; st['acc'] = o
            elif r0 == 0: st['l'] = st['l'] + ls; st['acc'] = st['acc'] + o
            else:
                st['l'] = jnp.concatenate([st['l'][:r0], st['l'][r0:] + ls], axis=0)
                st['acc'] = jnp.concatenate([st['acc'][:r0], st['acc'][r0:] + o], axis=0)
        return f

    def fin(i):
        def f():
            st = sts[i]
            l = st['l']
            r = pltpu.reciprocal(l, approx=True); r = r * (2.0 - l * r)
            ctx[h, i * bq:(i + 1) * bq, :] = (st['acc'] * r).astype(BF16)
        return f
    for t in tiles(0): steps.append((('qk', 0), qk(0, t)))
    for i in range(nq):
        steps.append((('begin', i), begin(i)))
        tn = tiles(i + 1) if i + 1 < nq else []; tc = tiles(i)
        for j in range(max(len(tn), len(tc))):
            if j < len(tn): steps.append((('qk', i + 1), qk(i + 1, tn[j])))
            if j < len(tc): steps.append((('pv', i, j), pv(i, tc[j], j)))
        steps.append((('fin', i), fin(i)))
    return steps


def proj_steps(par, slot, xi, ci, wc, wslot, qb, kb, vb, rc):
    def half(w32):
        w = (w32 << 16) if par == 0 else (w32 & jnp.uint32(0xffff0000))
        return pltpu.bitcast(w, F32).astype(BF16)
    st = {}
    steps = []

    def getw():
        if 'wq' not in st:
            st['wq'] = half(wc[wslot, 0:M, :])
            st['wkv'] = jnp.concatenate([half(wc[wslot, M:M + C, :]), half(wc[wslot, M + C:, :])], axis=1)

    def qchunk(r):
        def f():
            getw()
            lhs = jnp.concatenate([bf(xi[j, r * rc // 2:(r + 1) * rc // 2, :]) for j in range(M // 128)], axis=1)
            q = jnp.dot(lhs, st['wq'], preferred_element_type=F32) * (D ** -0.5 * LOG2E)
            qb[slot, r * rc:(r + 1) * rc, :] = q.astype(BF16)
        return f

    def kvchunk(r):
        def f():
            getw()
            lhs = jnp.concatenate([bf(ci[j, r * rc // 2:(r + 1) * rc // 2, :]) for j in range(C // 128)], axis=1)
            kv = jnp.dot(lhs, st['wkv'], preferred_element_type=F32)
            kb[slot, r * rc:(r + 1) * rc, :] = kv[:, :D].astype(BF16)
            vb[slot, r * rc:(r + 1) * rc, :] = kv[:, D:].astype(BF16)
        return f
    for r in range(S // rc):
        steps.append(kvchunk(r)); steps.append(qchunk(r))
    return steps


SCOPES = False
DYN_A = tuple(range(8, 16))
OUT_INLINE = False
_stack = []
def begin_scope(n):
    if SCOPES:
        sc = jax.named_scope(n); sc.__enter__(); _stack.append(sc)
def end_scope():
    if SCOPES:
        _stack.pop().__exit__(None, None, None)


def b_steps(R, UR):
    r2 = float(np.sqrt(0.5))
    HI = jnp.uint32(0xffff0000)
    fi = R.fs.bitcast(jnp.int32); gi = R.gs.bitcast(jnp.int32); mai = R.mas.bitcast(jnp.int32)
    x1ri = R.x1r.bitcast(jnp.int32); x1ii = R.x1i.bitcast(jnp.int32)

    def p1(a):
        m, par = a // 2, a % 2

        def f():
            xa = []
            for A in range(8):
                w = R.bxs[m, :, A * 128:(A + 1) * 128]
                xa.append(pltpu.bitcast(w << 16 if par == 0 else w & HI, F32))
            u0, u1 = xa[0] + xa[4], xa[0] - xa[4]; u2, u3 = xa[2] + xa[6], xa[2] - xa[6]
            u4, u5 = xa[1] + xa[5], xa[1] - xa[5]; u6, u7 = xa[3] + xa[7], xa[3] - xa[7]
            s_, t_ = u0 + u2, u4 + u6
            d57, s57 = (u5 - u7) * r2, (u5 + u7) * r2
            L = [(s_ + t_, s_ - t_), (u1 + d57, (u3 + s57) * -1.0), (u0 - u2, u6 - u4), (u1 - d57, u3 - s57)]
            for j in range(4):
                data = jnp.concatenate(L[j], axis=1).astype(BF16)
                nr = 272 if j == 0 else 256
                lhs = jnp.concatenate([bf(fi[j, 0, 0:nr // 2, :]), bf(fi[j, 1, 0:nr // 2, :])], axis=1)
                o = lax.dot_general(lhs, data, NT, preferred_element_type=F32).astype(BF16)
                R.x1r[a, j * 128:(j + 1) * 128, :] = o[:128]
                R.x1i[a, j * 128:(j + 1) * 128, :] = o[128:256]
                if j == 0:
                    R.x1r[a, 512:528, :] = o[256:272]
        return f

    def p2(a, k0, k1):
        def f():
            lhs = jnp.concatenate([bf(x1ri[a, k0 // 2:k1 // 2, :]), bf(x1ii[a, k0 // 2:k1 // 2, :])], axis=1)
            rhs = jnp.concatenate([bf(mai[a, 0]), bf(mai[a, 1])], axis=1)
            o = jnp.dot(lhs, rhs, preferred_element_type=F32)
            for t in range(k0 // 128, (k1 + 127) // 128):
                l0 = max(k0, t * 128); l1 = min(k1, (t + 1) * 128)
                R.vt[t][0, a, l0 - t * 128:l1 - t * 128, :] = o[l0 - k0:l1 - k0, :128]
                R.vt[t][1, a, l0 - t * 128:l1 - t * 128, :] = o[l0 - k0:l1 - k0, 128:]
        return f

    def mid(k0):
        if True:
            j, rem = k0 // 128, k0 % 128
            hf, e0 = rem // 64, rem % 64
            c = (0, 4)[hf] if j == 0 else (j, 8 - j)[hf]

            def wload(cc):
                wr_ = R.wr32[cc, pl.ds(c // 2 + 4 * e0, UR, stride=4), :]
                wi_ = R.wi32[cc, pl.ds(c // 2 + 4 * e0, UR, stride=4), :]
                if c % 2 == 0:
                    return pltpu.bitcast(wr_ << 16, F32), pltpu.bitcast(wi_ << 16, F32)
                return pltpu.bitcast(wr_ & HI, F32), pltpu.bitcast(wi_ & HI, F32)
        def cmul(x, w):
            return (x[0] * w[0] - x[1] * w[1], x[0] * w[1] + x[1] * w[0])

        def f():
            t, kk = k0 // 128, k0 % 128
            xs_ = [((R.vt[t][R.z0, a, kk:kk + UR, :], R.vt[t][R.z0 + 1, a, kk:kk + UR, :]) if a in DYN_A else
                    (R.vt[t][0, a, kk:kk + UR, :], R.vt[t][1, a, kk:kk + UR, :])) for a in range(16)]
            X = fft16(xs_, False)
            Y = [cmul(X[cc], wload(cc)) for cc in range(16)]
            if k0 == 0:
                xn = [(R.vt[4][0, a, 0:UR, :], R.vt[4][1, a, 0:UR, :]) for a in range(16)]
                XN = fft16(xn, False)
                YN = [cmul(XN[cc], (jnp.broadcast_to(R.wn[0, :, cc * 128:(cc + 1) * 128].astype(F32), (UR, 128)),
                                    jnp.broadcast_to(R.wn[1, :, cc * 128:(cc + 1) * 128].astype(F32), (UR, 128))))
                      for cc in range(16)]
                ln = lax.broadcasted_iota(jnp.int32, (UR, 128), 1)
                rw = lax.broadcasted_iota(jnp.int32, (UR, 128), 0)
                idx = (128 - ln) & 127
                Pm = [(jnp.take_along_axis(Y[c][0] + YN[c][1], idx, axis=1),
                       jnp.take_along_axis(Y[c][1] - YN[c][0], idx, axis=1)) for c in range(16)]
                Y2 = []
                for cc in range(16):
                    fr_ = jnp.where(ln == 0, Pm[(16 - cc) % 16][0], Pm[15 - cc][0])
                    fi2 = jnp.where(ln == 0, Pm[(16 - cc) % 16][1], Pm[15 - cc][1])
                    tr_ = (Y[cc][0] - YN[cc][1] + fr_) * 0.5
                    ti_ = (Y[cc][1] + YN[cc][0] - fi2) * 0.5
                    Y2.append((jnp.where(rw == 0, tr_, Y[cc][0]), jnp.where(rw == 0, ti_, Y[cc][1])))
                Y = Y2
            Tt = fft16(Y, True)
            for a in range(16):
                R.vt[t][2, a, kk:kk + UR, :] = Tt[a][0]
                R.vt[t][3, a, kk:kk + UR, :] = Tt[a][1]
        return f

    def p3(a, t):
        def f():
            lhs = jnp.concatenate([bf(mai[a, 0]), bf(mai[a, 1])], axis=1)
            data = jnp.concatenate([R.vt[t][2, a], R.vt[t][3, a]], axis=1).astype(BF16)
            o = lax.dot_general(lhs, data, NT, preferred_element_type=F32)
            R.y1r[a, :, t * 128:(t + 1) * 128] = o[:128]
            R.y1i[a, :, t * 128:(t + 1) * 128] = o[128:]
        return f

    lane = lax.broadcasted_iota(jnp.int32, (128, 128), 1)
    st = {}

    def p4(a):
        def f():
            U = []
            for j in range(4):
                yr = R.y1r[a, :, j * 128:(j + 1) * 128]; yi = R.y1i[a, :, j * 128:(j + 1) * 128]
                lhs = jnp.concatenate([yr, yi], axis=1).astype(BF16)
                rhs = jnp.concatenate([bf(gi[j, 0]), bf(gi[j, 1])], axis=1)
                o = jnp.dot(lhs, rhs, preferred_element_type=F32)
                U.append((o[:, :128], o[:, 128:]))
            T0, T4 = U[0]; U1r, U1i = U[1]; U2r, U2i = U[2]; U3r, U3i = U[3]
            P, Q = T0 + T4, T0 - T4
            A_, B_ = P + U2r, P - U2r
            s13 = U1r + U3r; d = U3i - U1i
            Qm, Qp = Q - U2i, Q + U2i
            t1, t2 = U1r - U3r, U1i + U3i
            e1, e3 = (t1 - t2) * r2, (t1 + t2) * r2
            st[a] = [A_ + s13, Qm + e1, B_ + d, Qp - e3, A_ - s13, Qm - e1, B_ - d, Qp + e3]
            if a % 2 == 1:
                m = a // 2
                for A in range(8):
                    R.bxs[m, :, A * 128:(A + 1) * 128] = pltpu.bitcast(
                        pltpu.pack_elementwise([st[a - 1][A], st[a][A]], packed_dtype=BF16), jnp.uint32)
                if R.out_inline: R.b_out[m].start()
        return f
    return p1, p2, mid, p3, p4


class NS:
    pass


def kernel(z_ref, x_hbm, c_hbm, wq_hbm, wk_hbm, wv_hbm, wo_hbm, bx_hbm, wr_hbm, wi_hbm, f_hbm, g_hbm, e_hbm, tw_hbm,
           out_hbm,
           xs, cs, wc, qb, kb, vb, ctx, wos, bxs, wr32, wi32, wn, x1r, x1i, vt, y1r, y1i,
           fs, gs, mas, es, tws, ost,
           sem, wsem, osem, *, UR, bq, bk, rc, RO, border, doA=True):
    def cp(src, dst, s): return pltpu.make_async_copy(src, dst, s)
    bx_u = bx_hbm.bitcast(jnp.uint32)
    bx_cp = [cp(bx_u.at[:, m, :], bxs.at[m], sem.at[m]) for m in range(8)]
    f_cp = cp(f_hbm, fs, sem.at[8])
    e_cp = [cp(e_hbm, es, sem.at[9]), cp(tw_hbm, tws, sem.at[10])]
    g_cp = cp(g_hbm, gs, sem.at[11])
    wr_u = wr_hbm.at[pl.ds(0, 512), :].bitcast(jnp.uint32)
    wi_u = wi_hbm.at[pl.ds(0, 512), :].bitcast(jnp.uint32)
    w_cp = [cp(wr_u.at[:, cc * 128:(cc + 1) * 128], wr32.at[cc], sem.at[36 + cc]) for cc in range(16)]
    w_cp += [cp(wi_u.at[:, cc * 128:(cc + 1) * 128], wi32.at[cc], sem.at[52 + cc]) for cc in range(16)]
    wn_cp = [cp(wr_hbm.at[pl.ds(512, 1), :], wn.at[0], sem.at[12]), cp(wi_hbm.at[pl.ds(512, 1), :], wn.at[1], sem.at[13])]
    x_cp = [cp(x_hbm.at[:, a * 128:(a + 1) * 128], xs.at[a], sem.at[14 + a]) for a in range(8)]
    c_cp = [cp(c_hbm.at[:, a * 128:(a + 1) * 128], cs.at[a], sem.at[22 + a]) for a in range(4)]
    wo_cp = [cp(wo_hbm.at[:, a * 128:(a + 1) * 128], wos.at[a], sem.at[26 + a]) for a in range(8)]
    wq_u = wq_hbm.bitcast(jnp.uint32); wk_u = wk_hbm.bitcast(jnp.uint32); wv_u = wv_hbm.bitcast(jnp.uint32)
    out_u = out_hbm.bitcast(jnp.uint32)
    b_out = [cp(bxs.at[m], out_u.at[:, m, pl.ds(DM, DM)], osem.at[m]) for m in range(8)]

    def w_cps(j, wslot):
        return [cp(wq_u.at[:, j, :], wc.at[wslot, pl.ds(0, M), :], wsem.at[wslot, 0]),
                cp(wk_u.at[:, j, :], wc.at[wslot, pl.ds(M, C), :], wsem.at[wslot, 1]),
                cp(wv_u.at[:, j, :], wc.at[wslot, pl.ds(M + C, C), :], wsem.at[wslot, 2])]
    R = NS()
    R.z0 = z_ref[0]
    R.out_inline = OUT_INLINE
    R.fs, R.gs, R.mas, R.x1r, R.x1i, R.vt = fs, gs, mas, x1r, x1i, vt
    R.bxs, R.wr32, R.wi32, R.wn, R.y1r, R.y1i, R.b_out = bxs, wr32, wi32, wn, y1r, y1i, b_out
    p1, p2, mid, p3, p4 = b_steps(R, UR)

    xi = xs.bitcast(jnp.int32); ci = cs.bitcast(jnp.int32)
    qi = qb.bitcast(jnp.int32); ki = kb.bitcast(jnp.int32); vi = vb.bitcast(jnp.int32)
    proj0 = proj_steps(0, 0, xi, ci, wc, 0, qb, kb, vb, rc)

    def start(ds): return lambda: [d.start() for d in ds]
    def wait(ds): return lambda: [d.wait() for d in ds]

    def zero_init():
        for a in range(16):
            x1i[a, pl.ds(512, 16), :] = jnp.zeros((16, 128), BF16)
    def gen_ma():
        for d in e_cp: d.wait()
        fr = es[0]; fi_ = es[1]
        for a in range(16):
            tr_ = jnp.broadcast_to(tws[a:a + 1, :], (128, 128)); ti_ = jnp.broadcast_to(tws[16 + a:17 + a, :], (128, 128))
            er = fr * tr_ - fi_ * ti_
            ei = fr * ti_ + fi_ * tr_
            erb = er.astype(BF16)
            mas[a, 0, 0:128, :] = erb
            mas[a, 1, 128:256, :] = erb
            mas[a, 1, 0:128, :] = ei.astype(BF16)
            mas[a, 0, 128:256, :] = (-ei).astype(BF16)
    E = dict(
        s_f=start([f_cp]), w_f=wait([f_cp]), s_ma=start(e_cp), w_ma=gen_ma,
        s_w=start(w_cp + wn_cp), s_wr=start(w_cp[:16] + wn_cp), s_wi=start(w_cp[16:]), w_w=wait(w_cp[:16] + wn_cp), w_w2=wait(w_cp[16:]), s_g=start([g_cp]), w_g=wait([g_cp]),
        s_c=start(c_cp), w_c=wait(c_cp), s_x=start(x_cp), w_x=wait(x_cp),
        s_w0=start(w_cps(0, 0)), w_w0=wait(w_cps(0, 0)), s_w1=start(w_cps(1, 1)), s_wo=start(wo_cp),
        w_w1=wait(w_cps(1, 1)), w_wo=wait(wo_cp),
        zero=zero_init, s_out=start(b_out), s_out_a=start(b_out[:4]), s_out_b=start(b_out[4:]))
    for m in range(8):
        E['s_bx%d' % m] = start([bx_cp[m]]); E['w_bx%d' % m] = wait([bx_cp[m]])

    begin_scope('B')

    def run_item(item):
        if isinstance(item, tuple) and item[0] == 'blk':
            @pl.when(R.z0 == 0)
            def _():
                for it in item[1]: run_item(it)
        elif isinstance(item, str):
            if item.startswith('scope:'):
                end_scope(); begin_scope(item[6:])
            else:
                E[item]()
        elif item[0] == 'p1': p1(item[1])()
        elif item[0] == 'p2': p2(*item[1:])()
        elif item[0] == 'mid': mid(item[1])()
        elif item[0] == 'p3': p3(*item[1:])()
        elif item[0] == 'p4': p4(item[1])()
        elif item[0] == 'proj': proj0[item[1]]()
        else: raise ValueError(item)
    for item in border(UR): run_item(item)
    end_scope()
    if not doA:
        if doA is not None:
            for d_ in b_out: d_.wait()
        return

    begin_scope('HEADS')

    def head(slot, h, proj):
        pi = 0
        for tag, f in attention_steps(qi, ki, vi, ctx, slot, h, bq, bk):
            f()
            if tag[0] == 'begin' and tag[1] in (0, S // bq - 1) and pi < len(proj):
                proj[pi](); pi += 1
        for f in proj[pi:]: f()

    def pair(p, wcur, wnext, last):
        pr = proj_steps(1, 1, xi, ci, wc, wcur, qb, kb, vb, rc)
        head(0, 2 * p, pr[1::2] + pr[0::2])
        pr = [] if last else proj_steps(0, 0, xi, ci, wc, wnext, qb, kb, vb, rc)
        head(1, 2 * p + 1, pr[1::2] + pr[0::2])

    def body(p, _):
        wcur = lax.rem(p, 3); wnext = lax.rem(p + 1, 3)
        for d in w_cps(p + 1, wnext): d.wait()
        for d in w_cps(jnp.minimum(p + 2, H // 2 - 1), lax.rem(p + 2, 3)): d.start()
        pair(p, wcur, wnext, False)
        return 0
    lax.fori_loop(0, H // 2 - 1, body, 0)
    for d in w_cps(0, (H // 2) % 3): d.wait()
    end_scope()
    begin_scope('LAST')
    pair(H // 2 - 1, (H // 2 - 1) % 3, 0, True)

    end_scope()
    begin_scope('OUT')
    for d in wo_cp: d.wait()
    for d_ in b_out: d_.wait()
    ctxi = ctx.bitcast(jnp.int32); woi = wos.bitcast(jnp.int32)

    def a_out_cps(r16, osl):
        return [cp(ost.at[osl, a], out_hbm.at[pl.ds(r16, RO // 16), :, pl.ds(a * 128, 128)], osem.at[8 + osl * 8 + a]) for a in range(8)]

    def obody(r, _):
        r0 = r * (RO // 16); h0 = pl.multiple_of(r * (RO // 2), RO // 2)
        osl = r & 1

        @pl.when(r >= 2)
        def _():
            for d_ in a_out_cps(r0 - 2 * (RO // 16), osl): d_.wait()
        lhs = jnp.concatenate([bf(ctxi[hh, pl.ds(h0, RO // 2), :]) for hh in range(H)], axis=1)
        rhs = jnp.concatenate([bf(woi[a]) for a in range(8)], axis=1)
        o = jnp.dot(lhs, rhs, preferred_element_type=F32)
        for a in range(8):
            ost[osl, a] = o[:, a * 128:(a + 1) * 128].astype(BF16).reshape(RO // 16, 16, 128)
        for d_ in a_out_cps(r0, osl): d_.start()
        return 0
    lax.fori_loop(0, S // RO, obody, 0)
    for r in (S // RO - 2, S // RO - 1):
        for d_ in a_out_cps(r * (RO // 16), r & 1): d_.wait()
    end_scope()


def inter(*lists):
    lists = [l for l in lists if l]; it = []
    for li, l in enumerate(lists):
        for k, x in enumerate(l): it.append(((k + 0.5) / len(l), li, x))
    it.sort(key=lambda t: (t[0], t[1]))
    return [x for _, _, x in it]


def timed_border(mid_rate=130.0, mid_start=4500, p4proj=True):
    def border(UR):
        o = ['s_bx0', 's_ma', 's_f', 's_bx1', 's_bx2', 'zero', 'w_ma', 's_bx3', 'w_f']
        for m in range(8):
            o += ['w_bx%d' % m, ('p1', 2 * m), ('p1', 2 * m + 1)]
            if m == 0: o += ['s_bx4', 's_bx5']
            if m == 1: o += ['s_bx6', 's_bx7']
            if m == 2: o += ['s_wr']
            if m == 3: o += ['s_wi']
        o += ['scope:P2']
        items = []; t = 0.0
        for a in range(16): items.append((t, ('p2', a, 512, 528))); t += 20
        for tt in range(4):
            for a in range(16): items.append((t, ('p2', a, tt * 128, (tt + 1) * 128))); t += 128
        tm = mid_start; last = {}
        for k0 in range(0, 512, UR):
            items.append((tm, ('mid', k0))); last[k0 // 128] = tm; tm += mid_rate * UR / 8
        for tt in range(4):
            t = max(t, last[tt] + 1)
            for a in range(16): items.append((t, ('p3', a, tt))); t += 128
        items.sort(key=lambda x: x[0])
        seq = [x for _, x in items]; pos = {x: i for i, x in enumerate(seq)}
        for x in seq:
            if x[0] == 'mid': assert pos[x] > max(pos[y] for y in seq if y[0] == 'p2' and y[2] == x[1] // 128 * 128)
            if x[0] == 'p3': assert pos[x] > max(pos[y] for y in seq if y[0] == 'mid' and y[1] // 128 == x[2])
        for _, x in items:
            if x == ('mid', 0): o += ['scope:WW', 'w_w', 's_g', 's_c', 's_w0', 's_x', 'w_w2', 'scope:S']
            o.append(x)
        o += ['scope:WX', 'w_g', 'w_c', 'w_w0', 'w_x', 's_w1', 's_wo', 'scope:P4']
        proj = [('proj', i) for i in range(16)]
        if p4proj: o += inter([('p4', a) for a in range(16)], proj)
        else: o += [('p4', a) for a in range(16)] + proj
        o += ['s_out']
        return o
    return border


def make_fn(scopes=False, UR=8, bq=256, bk=768, rc=256, RO=256, border=None, tdtype=BF16, doA=True):
    global SCOPES
    SCOPES = scopes
    FTb, Gb, F128, TW = _consts()
    if border is None: border = timed_border()

    def fn(A_x, A_c_kv, A_w_q, A_w_uk, A_w_uv, A_w_o, B_x, B_w_r, B_w_i):
        x = A_x.reshape(S, M); c = A_c_kv.reshape(S, C); wo = A_w_o.reshape(H * D, M)
        bx = B_x.reshape(128, 16, DM)
        out = pl.pallas_call(
            functools.partial(kernel, UR=UR, bq=bq, bk=bk, rc=rc, RO=RO, border=border, doA=doA),
            in_specs=[pl.BlockSpec(memory_space=pltpu.SMEM)] + [pl.BlockSpec(memory_space=pl.ANY)] * 13,
            out_specs=pl.BlockSpec(memory_space=pl.ANY),
            out_shape=jax.ShapeDtypeStruct((128, 16, M + DM), BF16),
            scratch_shapes=[
                pltpu.VMEM((M // 128, S, 128), BF16),
                pltpu.VMEM((C // 128, S, 128), BF16),
                pltpu.VMEM((3, M + 2 * C, D), jnp.uint32),
                pltpu.VMEM((2, S, D), BF16), pltpu.VMEM((2, S, D), BF16), pltpu.VMEM((2, S, D), BF16),
                pltpu.VMEM((H, S, D), BF16),
                pltpu.VMEM((8, H * D, 128), BF16),
                pltpu.VMEM((8, 128, DM), jnp.uint32),
                pltpu.VMEM((16, 256, 128), jnp.uint32), pltpu.VMEM((16, 256, 128), jnp.uint32),
                pltpu.VMEM((2, 1, S), BF16),
                pltpu.VMEM((16, 528, 128), BF16), pltpu.VMEM((16, 528, 128), BF16),
                [pltpu.VMEM((4, 16, 128, 128), F32) for t in range(4)] + [pltpu.VMEM((2, 16, 16, 128), F32)],
                pltpu.VMEM((16, 128, 512), F32), pltpu.VMEM((16, 128, 512), F32),
                pltpu.VMEM((4, 2, 272, 128), BF16), pltpu.VMEM((4, 2, 256, 128), BF16),
                pltpu.VMEM((16, 2, 256, 128), BF16),
                pltpu.VMEM((2, 128, 128), F32), pltpu.VMEM((32, 128), F32),
                pltpu.VMEM((2, 8, RO // 16, 16, 128), BF16),
                pltpu.SemaphoreType.DMA((68,)), pltpu.SemaphoreType.DMA((3, 3)), pltpu.SemaphoreType.DMA((24,)),
            ],
            compiler_params=pltpu.CompilerParams(vmem_limit_bytes=126 * 2 ** 20),
        )(jnp.zeros((1,), jnp.int32), x, c, A_w_q, A_w_uk, A_w_uv, wo, bx, B_w_r.T, B_w_i.T,
          jnp.asarray(FTb), jnp.asarray(Gb), jnp.asarray(F128), jnp.asarray(TW))
        return out.reshape(1, S, M + DM)
    return fn


_fn = make_fn()


@jax.jit
def pallas_concat_heads__compressed_kv_cla__spectral_gfnet__prompt_kernel(
    A_x: jax.Array,
    A_c_kv: jax.Array,
    A_w_q: jax.Array,
    A_w_uk: jax.Array,
    A_w_uv: jax.Array,
    A_w_o: jax.Array,
    B_x: jax.Array,
    B_w_r: jax.Array,
    B_w_i: jax.Array,
):
    return _fn(A_x, A_c_kv, A_w_q, A_w_uk, A_w_uv, A_w_o, B_x, B_w_r, B_w_i)
```
